```python
import jax
import jax.numpy as jnp

def _softmax(x, axis=-1):
    return jax.nn.softmax(x, axis=axis)

def _gelu(x):
    return jax.nn.gelu(x, approximate=True)

def _silu(x):
    return jax.nn.silu(x)

def _sigmoid(x):
    return jax.nn.sigmoid(x)

def _layernorm(x, axis=-1, eps=1e-05):
    m = jnp.mean(x, axis=axis, keepdims=True)
    v = jnp.var(x, axis=axis, keepdims=True)
    return (x - m) / jnp.sqrt(v + eps)

def _scatter_add(tgt, idx, src, axis=0):
    return tgt.at[idx].add(src)

def _segment_sum(src, seg, n):
    return jax.ops.segment_sum(src, seg, n)

class _Rng:

    def __init__(self, key):
        self._k = key

    def _next(self):
        self._k, sub = jax.random.split(self._k)
        return sub

    def normal(self, shape):
        return jax.random.normal(self._next(), shape, dtype=jnp.bfloat16)

    def randint(self, lo, hi, shape):
        return jax.random.randint(self._next(), shape, lo, hi, dtype=jnp.int32)

    def uniform(self, shape, lo=0.0, hi=1.0):
        return jax.random.uniform(self._next(), shape, jnp.bfloat16, lo, hi)

    def permutation(self, n):
        return jax.random.permutation(self._next(), n)
kernel_name = 'concat_heads__memory_aug_recurrent_mem_tr__compressed_kv_cla__prompt'

def setup_inputs():
    _rng = _Rng(jax.random.key(int.from_bytes(__import__("os").urandom(4), "little")))
    _w = lambda a: (lambda t: t.astype(jnp.bfloat16) if jnp.issubdtype(t.dtype, jnp.floating) else t)(jnp.asarray(a))

    def _A_setup():
        B, S, Dm = (1, 2048, 448)
        H, Dh = (16, 256)
        M, seg = (8, 32)
        seg = min(seg, S)
        S = S // seg * seg
        return {'x': _w((lambda *s: _rng.normal(s) * 0.05)(B, S, Dm)), 'mem0': _w((lambda *s: _rng.normal(s) * 0.05)(B, M, Dm)), 'Wq': _w((lambda *s: _rng.normal(s) * 0.05)(Dm, H, Dh) * Dm ** (-0.5)), 'Wk': _w((lambda *s: _rng.normal(s) * 0.05)(Dm, H, Dh) * Dm ** (-0.5)), 'Wv': _w((lambda *s: _rng.normal(s) * 0.05)(Dm, H, Dh) * Dm ** (-0.5)), 'Wo': _w((lambda *s: _rng.normal(s) * 0.05)(H, Dh, Dm) * (H * Dh) ** (-0.5)), 'seg_len': seg}
    _A_in = _A_setup()

    def _B_setup():
        B, H, Sq, Sk, D, M = (1, 16, 2048, 2048, 256, 448)
        Dc = 4 * D
        return {'x': _w((lambda *s: _rng.normal(s) * 0.05)(B, Sq, M)), 'c_kv': _w((lambda *s: _rng.normal(s) * 0.05)(B, Sk, Dc)), 'w_q': _w((lambda *s: _rng.normal(s) * 0.05)(M, H, D) * M ** (-0.5)), 'w_uk': _w((lambda *s: _rng.normal(s) * 0.05)(Dc, H, D) * Dc ** (-0.5)), 'w_uv': _w((lambda *s: _rng.normal(s) * 0.05)(Dc, H, D) * Dc ** (-0.5)), 'w_o': _w((lambda *s: _rng.normal(s) * 0.05)(H, D, M) * (H * D) ** (-0.5))}
    _B_in = _B_setup()
    return {'A_x': _A_in['x'], 'A_mem0': _A_in['mem0'], 'A_Wq': _A_in['Wq'], 'A_Wk': _A_in['Wk'], 'A_Wv': _A_in['Wv'], 'A_Wo': _A_in['Wo'], 'A_seg_len': _A_in['seg_len'], 'B_x': _B_in['x'], 'B_c_kv': _B_in['c_kv'], 'B_w_q': _B_in['w_q'], 'B_w_uk': _B_in['w_uk'], 'B_w_uv': _B_in['w_uv'], 'B_w_o': _B_in['w_o']}

def reference(A_x, A_mem0, A_Wq, A_Wk, A_Wv, A_Wo, A_seg_len, B_x, B_c_kv, B_w_q, B_w_uk, B_w_uv, B_w_o):

    def _A_ref(x, mem0, Wq, Wk, Wv, Wo, seg_len):
        B, S, Dm = x.shape
        H, Dh = (Wq.shape[1], Wq.shape[2])
        M = mem0.shape[1]
        scale = Dh ** (-0.5)
        n_seg = S // seg_len
        L = M + seg_len
        idx = jnp.arange(L)
        mask = (idx[:, None] < M) | (idx[:, None] >= idx[None, :])
        mem = mem0
        outs = []
        for s in range(n_seg):
            xs = x[:, s * seg_len:(s + 1) * seg_len, :].copy()
            h = jnp.concatenate([mem, xs], axis=1)
            q = jnp.einsum('btd,dhe->bhte', h, Wq)
            k = jnp.einsum('btd,dhe->bhte', h, Wk)
            v = jnp.einsum('btd,dhe->bhte', h, Wv)
            scores = jnp.einsum('bhqe,bhke->bhqk', q, k) * scale
            scores = jnp.where(mask[None, None], scores, -1000000000.0)
            p = _softmax(scores, axis=-1)
            o = jnp.einsum('bhqk,bhke->bhqe', p, v)
            o = jnp.einsum('bhte,hed->btd', o, Wo)
            mem = o[:, :M, :].copy()
            outs.append(o[:, M:, :])
        return jnp.concatenate(outs, axis=1)

    def _B_ref(x, c_kv, w_q, w_uk, w_uv, w_o):
        B, Sq, M = (x.shape[0], x.shape[1], x.shape[2])
        Sk = c_kv.shape[1]
        H, D = (w_q.shape[1], w_q.shape[2])
        q = jnp.einsum('bqm,mhd->bhqd', x, w_q)
        k = jnp.einsum('bkc,chd->bhkd', c_kv, w_uk)
        v = jnp.einsum('bkc,chd->bhkd', c_kv, w_uv)
        scores = jnp.einsum('bhqd,bhkd->bhqk', q, k) * D ** (-0.5)
        off = Sk - Sq
        qi = jnp.arange(Sq)[:, None]
        kj = jnp.arange(Sk)[None, :]
        cmask = kj <= qi + off
        scores = jnp.where(cmask[None, None], scores, -1000000000.0)
        p = _softmax(scores, axis=-1)
        ctx = jnp.einsum('bhqk,bhkd->bhqd', p, v)
        return jnp.einsum('bhqd,hdm->bqm', ctx, w_o)
    a = _A_ref(A_x, A_mem0, A_Wq, A_Wk, A_Wv, A_Wo, A_seg_len)
    b = _B_ref(B_x, B_c_kv, B_w_q, B_w_uk, B_w_uv, B_w_o)
    return jnp.concatenate([a, b], axis=-1)
```

```python
import functools
import math

import jax
import jax.numpy as jnp
from jax import lax
import jax.experimental.pallas as pl
import jax.experimental.pallas.tpu as pltpu

BF = jnp.bfloat16
F32 = jnp.float32
LOG2E = math.log2(math.e)
NEG_MASK = -1e9 * LOG2E
NEG_PAD = -3e38

NCHAIN = 4
WARM = 4
TB = 256
QB = 256


def _dot(a, b):
    return jnp.dot(a, b, preferred_element_type=F32)


def _dot_nt(a, b):
    return lax.dot_general(a, b, (((1,), (1,)), ((), ())), preferred_element_type=F32)


def _head_pair(raw_ref, j, m0, rows):
    u = raw_ref.bitcast(jnp.uint32)
    half = u.shape[0] // 2
    w = jnp.concatenate(
        [u.at[pl.ds(pl.multiple_of(i * half + m0 * 8, 8), rows * 8)][pl.ds(j, rows, stride=8), :]
         for i in range(2)], axis=1)
    lo = pltpu.bitcast(w << 16, F32).astype(BF)
    hi = pltpu.bitcast(w & jnp.uint32(0xFFFF0000), F32).astype(BF)
    return lo, hi


class _Load:
    def __init__(self, src, dst, sems, i):
        n = src.shape[0]
        if dst.shape != src.shape:
            self.cps = [pltpu.make_async_copy(src.at[:, 128 * k:128 * (k + 1)],
                                              dst.at[k * n:(k + 1) * n],
                                              sems.at[2 * i + k]) for k in range(2)]
        else:
            self.cps = [pltpu.make_async_copy(src, dst, sems.at[2 * i])]

    def start(self):
        for cp in self.cps:
            cp.start()

    def wait(self):
        for cp in self.cps:
            cp.wait()


def _merge_pair(e, o):
    return jnp.concatenate([e[:, :384], e[:, 384:] + o[:, :128], o[:, 128:]], axis=1)


def _softmax2(s):
    m = jnp.max(s, axis=-1, keepdims=True)
    p = jnp.exp2(s - m)
    return p * (1.0 / jnp.sum(p, axis=-1, keepdims=True))


def _kernel(xa_h, mem0_h, wq_h, wk_h, wv_h, wo_h, xb_h, c_h, wqb_h, wuk_h, wuv_h, wob_h,
            out_ref, xbt, xb, ckv, wqb, wuk, wuv, wob, wq_s, wk_s, wv_s, sems, *, S, DM, H, DH, MEM, SEG, DC):
    NP = H // 2
    NSEG = S // SEG
    STRIDE = (NSEG - WARM) // NCHAIN
    NPASS = WARM + STRIDE
    scale = DH ** -0.5 * LOG2E

    b_copies = [_Load(s, d, sems, 6 + i) for i, (s, d) in enumerate(
        [(c_h, ckv), (wuk_h, wuk), (wuv_h, wuv), (xb_h, xbt), (wqb_h, wqb), (wob_h, wob)])]

    def branch_a(xat, xa, mem0, wq, wk, wv, wo, a_all, b_all, keys, qp, ph):
        a_copies = [_Load(s, d, sems, i) for i, (s, d) in enumerate(
            [(wq_h, wq), (wk_h, wk), (wv_h, wv), (wo_h, wo), (xa_h, xat), (mem0_h, mem0)])]
        for cp in a_copies[:2]:
            cp.start()
        for cp in a_copies[:2]:
            cp.wait()
        for cp in a_copies[2:]:
            cp.start()

        for j in range(NP):
            q0, q1 = _head_pair(wq, j, 0, DM)
            k0, k1 = _head_pair(wk, j, 0, DM)
            z = jnp.zeros((64, DH), BF)
            a0 = _dot_nt(q0, jnp.concatenate([k0, z], axis=0))
            a1 = _dot_nt(q1, jnp.concatenate([z, k1], axis=0))
            a_all[j] = (_merge_pair(a0, a1) * scale).astype(BF)

        for cp in a_copies[2:]:
            cp.wait()
        for cp in b_copies:
            cp.start()

        for j in range(NP):
            v0, v1 = _head_pair(wv, j, 0, DM)
            z = jnp.zeros((64, DH), BF)
            b_all[j, 0:DM, :] = _dot_nt(v0, jnp.concatenate([wo[2 * j], z], 0)).astype(BF)
            b_all[j, DM:2 * DM, :] = _dot_nt(v1, jnp.concatenate([wo[2 * j + 1], z], 0)).astype(BF)

        def make_keys(b, _):
            r0 = pl.multiple_of(b * TB, TB)
            xt = xat[:, pl.ds(r0, TB)]
            z = jnp.zeros((64, TB), BF)
            xp = jnp.concatenate([xt, z], axis=0).T
            xs = jnp.concatenate([z, xt], axis=0).T
            xa[pl.ds(r0, TB), :] = xp
            z = jnp.zeros((16, 512), BF)
            for g in range(TB // SEG):
                s = b * (TB // SEG) + g
                keys[s, 16:48, :] = xp[g * SEG:(g + 1) * SEG]
                keys[s, 48:64, :] = z
                keys[s, 80:112, :] = xs[g * SEG:(g + 1) * SEG]
                keys[s, 112:128, :] = z
        lax.fori_loop(0, S // TB, make_keys, None)

        row = lax.broadcasted_iota(jnp.int32, (128, 128), 0)
        col = lax.broadcasted_iota(jnp.int32, (128, 128), 1)
        kk = col - jnp.where(row >= 64, 64, 0)
        mem_valid = ((kk >= 0) & (kk < MEM)) | ((kk >= 16) & (kk < 16 + SEG))

        def one_pass(t, carry):
            mem, spec = carry
            spec = jnp.where(t == WARM, mem, spec)
            sh = pltpu.roll(mem, 64, 1)
            z8 = jnp.zeros((8, 512), F32)
            for c in range(NCHAIN):
                seg = c * STRIDE + t
                keys[seg, 0:16, :] = jnp.concatenate([mem[8 * c:8 * c + 8], z8], 0).astype(BF)
                keys[seg, 64:80, :] = jnp.concatenate([sh[8 * c:8 * c + 8], z8], 0).astype(BF)
            mb = mem[:, :DM].astype(BF)
            qs = [_dot(mb, a_all[j]) for j in range(NP)]
            phs = []
            for c in range(NCHAIN):
                kc = keys[c * STRIDE + t]
                lhs = jnp.concatenate(
                    [q[8 * c:8 * c + 8, 0:512] for q in qs]
                    + [q[8 * c:8 * c + 8, 384:896] for q in qs], axis=0).astype(BF)
                s = jnp.where(mem_valid, _dot_nt(lhs, kc), NEG_PAD)
                r = _dot(_softmax2(s).astype(BF), kc)
                phs.append([_merge_pair(r[8 * j:8 * j + 8], r[64 + 8 * j:72 + 8 * j])
                            for j in range(NP)])
            new = None
            for j in range(NP):
                l = jnp.concatenate([phs[c][j] for c in range(NCHAIN)], axis=0).astype(BF)
                d = _dot(l, b_all[j])
                new = d if new is None else new + d
            return new.astype(BF).astype(F32), spec

        def sweep(state):
            n, _, mem = state
            fin, spec = lax.fori_loop(jnp.where(n == 0, 0, WARM), NPASS, one_pass, (mem, mem))
            nxt = jnp.concatenate([spec[0:8], fin[0:8 * (NCHAIN - 1)]], axis=0)
            diff = pltpu.bitcast(nxt, jnp.int32) != pltpu.bitcast(spec, jnp.int32)
            return n + 1, jnp.max(diff.astype(jnp.int32)), nxt

        m0 = jnp.concatenate([mem0[...].astype(F32), jnp.zeros((MEM, 64), F32)], axis=1)
        lax.while_loop(lambda st: (st[0] < NCHAIN) & (st[1] > 0), sweep,
                       (jnp.int32(0), jnp.int32(1), jnp.concatenate([m0] * NCHAIN, axis=0)))

        trow = lax.broadcasted_iota(jnp.int32, (512, 128), 0)
        tcol = lax.broadcasted_iota(jnp.int32, (512, 128), 1)
        tk = tcol - jnp.where(trow >= 256, 64, 0)
        exists = ((tk >= 0) & (tk < MEM)) | ((tk >= 16) & (tk < 16 + SEG))
        visible = ((tk >= 0) & (tk < MEM)) | ((tk >= 16) & (tk - 16 <= (trow & (SEG - 1))))
        fill = jnp.where(exists, NEG_MASK, NEG_PAD).astype(F32)

        for cp in b_copies:
            cp.wait()

        def tok_block(b, _):
            for raw, dst, n in ((wqb, wq_s, DM), (wuk, wk_s, DC), (wuv, wv_s, DC)):
                rows = n // (S // TB)
                m0 = pl.multiple_of(b * rows, 8)
                for j in range(NP):
                    lo, hi = _head_pair(raw, j, m0, rows)
                    dst[2 * j, pl.ds(m0, rows), :] = lo
                    dst[2 * j + 1, pl.ds(m0, rows), :] = hi
            r0 = pl.multiple_of(b * TB, TB)
            xb[pl.ds(r0, TB), :] = jnp.concatenate(
                [xbt[:, pl.ds(r0, TB)], jnp.zeros((64, TB), BF)], axis=0).T
            x = xa[pl.ds(r0, TB), 0:DM]
            for j in range(NP):
                qp[j] = _dot(x, a_all[j]).astype(BF)
            for g in range(TB // SEG):
                kc = keys[b * (TB // SEG) + g]
                rows = slice(g * SEG, (g + 1) * SEG)
                lhs = jnp.concatenate(
                    [qp[j, rows, 0:512] for j in range(NP)]
                    + [qp[j, rows, 384:896] for j in range(NP)], axis=0)
                s = jnp.where(visible, _dot_nt(lhs, kc), fill)
                r = _dot(_softmax2(s).astype(BF), kc)
                for j in range(NP):
                    ph[j, rows, :] = _merge_pair(
                        r[32 * j:32 * j + 32], r[256 + 32 * j:288 + 32 * j]).astype(BF)
            acc = None
            for j in range(NP):
                d = _dot(ph[j], b_all[j])
                acc = d if acc is None else acc + d
            out_ref[pl.ds(r0, TB), 0:512] = acc.astype(BF)
        lax.fori_loop(0, S // TB, tok_block, None)

    pl.run_scoped(
        branch_a,
        pltpu.VMEM((DM, S), BF), pltpu.VMEM((S, 512), BF), pltpu.VMEM((MEM, DM), BF),
        pltpu.VMEM((2 * DM * H, 128), BF), pltpu.VMEM((2 * DM * H, 128), BF),
        pltpu.VMEM((2 * DM * H, 128), BF), pltpu.VMEM((H, DM, DH), BF),
        pltpu.VMEM((NP, DM, 2 * DM), BF), pltpu.VMEM((NP, 2 * DM, 512), BF),
        pltpu.VMEM((NSEG, 128, 512), BF),
        pltpu.VMEM((NP, TB, 2 * DM), BF), pltpu.VMEM((NP, TB, 2 * DM), BF))

    def branch_b(ctx, q_s, k_s, v_s):
        qi = lax.broadcasted_iota(jnp.int32, (QB, QB), 0)
        kj = lax.broadcasted_iota(jnp.int32, (QB, QB), 1)
        causal = kj <= qi

        def head(h, _):
            q_s[...] = (_dot(xb[:, 0:DM], wq_s[h]) * scale).astype(BF)
            k_s[...] = _dot(ckv[...], wk_s[h]).astype(BF)
            v_s[...] = _dot(ckv[...], wv_s[h]).astype(BF)
            for i in range(S // QB):
                q = q_s[i * QB:(i + 1) * QB, :]
                sd = jnp.where(causal, _dot_nt(q, k_s[i * QB:(i + 1) * QB, :]), NEG_MASK)
                m = jnp.max(sd, axis=-1, keepdims=True)
                if i:
                    so = _dot_nt(q, k_s[0:i * QB, :])
                    m = jnp.maximum(m, jnp.max(so, axis=-1, keepdims=True))
                pd = jnp.exp2(sd - m)
                l = jnp.sum(pd, axis=-1, keepdims=True)
                o = _dot(pd.astype(BF), v_s[i * QB:(i + 1) * QB, :])
                if i:
                    po = jnp.exp2(so - m)
                    l = l + jnp.sum(po, axis=-1, keepdims=True)
                    o = o + _dot(po.astype(BF), v_s[0:i * QB, :])
                ctx[h, i * QB:(i + 1) * QB, :] = (o * (1.0 / l)).astype(BF)
        lax.fori_loop(0, H, head, None)

        def out_block(i, _):
            r = pl.multiple_of(i * 512, 512)
            acc = None
            for h in range(H):
                d = _dot_nt(wob[h], ctx[h, pl.ds(r, 512), :])
                acc = d if acc is None else acc + d
            res = jnp.concatenate([jnp.zeros((64, 512), BF), acc.astype(BF)], axis=0).T
            lane = lax.broadcasted_iota(jnp.int32, (512, 128), 1)
            out_ref[pl.ds(r, 512), 384:512] = jnp.where(
                lane < 64, out_ref[pl.ds(r, 512), 384:512], res[:, 0:128])
            out_ref[pl.ds(r, 512), 512:896] = res[:, 128:512]
        lax.fori_loop(0, S // 512, out_block, None)

    pl.run_scoped(
        branch_b,
        pltpu.VMEM((H, S, DH), BF),
        pltpu.VMEM((S, DH), BF), pltpu.VMEM((S, DH), BF), pltpu.VMEM((S, DH), BF))


@functools.partial(jax.jit, static_argnames=("A_seg_len",))
def pallas_concat_heads__memory_aug_recurrent_mem_tr__compressed_kv_cla__prompt_kernel(
    A_x, A_mem0, A_Wq, A_Wk, A_Wv, A_Wo, A_seg_len,
    B_x, B_c_kv, B_w_q, B_w_uk, B_w_uv, B_w_o,
):
    _, S, DM = A_x.shape
    _, H, DH = A_Wq.shape
    MEM = A_mem0.shape[1]
    DC = B_c_kv.shape[2]
    assert (S, DM, H, DH, MEM, A_seg_len, DC) == (2048, 448, 16, 256, 8, 32, 1024)
    assert B_x.shape == A_x.shape and B_c_kv.shape[1] == S

    out = pl.pallas_call(
        functools.partial(_kernel, S=S, DM=DM, H=H, DH=DH, MEM=MEM, SEG=A_seg_len, DC=DC),
        out_shape=jax.ShapeDtypeStruct((S, 2 * DM), BF),
        in_specs=[pl.BlockSpec(memory_space=pl.ANY)] * 12,
        out_specs=pl.BlockSpec(memory_space=pltpu.VMEM),
        scratch_shapes=[
            pltpu.VMEM((DM, S), BF), pltpu.VMEM((S, 512), BF), pltpu.VMEM((S, DC), BF),
            pltpu.VMEM((2 * DM * H, 128), BF), pltpu.VMEM((2 * DC * H, 128), BF),
            pltpu.VMEM((2 * DC * H, 128), BF), pltpu.VMEM((H, DM, DH), BF),
            pltpu.VMEM((H, DM, DH), BF), pltpu.VMEM((H, DC, DH), BF), pltpu.VMEM((H, DC, DH), BF),
            pltpu.SemaphoreType.DMA((24,)),
        ],
        compiler_params=pltpu.CompilerParams(vmem_limit_bytes=120 * 1024 * 1024),
    )(
        A_x.reshape(S, DM).T, A_mem0.reshape(MEM, DM),
        A_Wq.reshape(DM * H, DH), A_Wk.reshape(DM * H, DH), A_Wv.reshape(DM * H, DH),
        A_Wo.transpose(0, 2, 1),
        B_x.reshape(S, DM).T, B_c_kv.reshape(S, DC),
        B_w_q.reshape(DM * H, DH), B_w_uk.reshape(DC * H, DH), B_w_uv.reshape(DC * H, DH),
        B_w_o.transpose(0, 2, 1),
    )
    return out.reshape(1, S, 2 * DM)
```

```python
import functools
import math

import jax
import jax.numpy as jnp
from jax import lax
import jax.experimental.pallas as pl
import jax.experimental.pallas.tpu as pltpu

BF = jnp.bfloat16
F32 = jnp.float32
LOG2E = math.log2(math.e)
NEG_MASK = -1e9 * LOG2E
NEG_PAD = -3e38

NCHAIN = 4
WARM = 4
TB = 128
QB = 256


def _dot(a, b):
    return jnp.dot(a, b, preferred_element_type=F32)


def _dot_nt(a, b):
    return lax.dot_general(a, b, (((1,), (1,)), ((), ())), preferred_element_type=F32)


def _split_heads(raw_ref, dst_ref, m0, rows, after=None, halves=(0, 1)):
    u = raw_ref.bitcast(jnp.uint32)
    half = u.shape[0] // 2
    g = rows // 8
    sub = lax.broadcasted_iota(jnp.int32, (g, 8, 128), 1)
    for i in halves:
        w = u[pl.ds(pl.multiple_of(i * half + m0 * 8, 64), rows * 8), :].reshape(g, 8, 8, 128)
        if after is not None:
            pins = jnp.stack([after.pop(0) for _ in range(g)])[:, None]
            w = w | ((pltpu.bitcast(pins, jnp.uint32) >> 31) >> 1)
        v = [w[:, m] for m in range(8)]
        for d in (4, 2, 1):
            keep = (sub & d) == 0
            for a in range(8):
                if not a & d:
                    x, y = v[a], v[a + d]
                    v[a] = jnp.where(keep, x, pltpu.roll(y, d, 1))
                    v[a + d] = jnp.where(keep, pltpu.roll(x, 8 - d, 1), y)
        for p in range(8):
            x = v[p].reshape(rows, 128)
            lo = pltpu.bitcast(x << 16, F32).astype(BF)
            hi = pltpu.bitcast(x & jnp.uint32(0xFFFF0000), F32).astype(BF)
            dst_ref[2 * p, pl.ds(m0, rows), 128 * i:128 * (i + 1)] = lo
            dst_ref[2 * p + 1, pl.ds(m0, rows), 128 * i:128 * (i + 1)] = hi


def _packed(*shape):
    return pltpu.VMEM(shape[:-2] + (shape[-2] // 2, shape[-1]), jnp.uint32)


def _as_bf16(*refs):
    return [r.bitcast(BF) for r in refs]


class _Load:
    def __init__(self, src, dst, sems, i, r0=0, rows=None):
        n = src.shape[0]
        rows = rows or n
        if dst.shape != src.shape:
            self.cps = [pltpu.make_async_copy(src.at[r0:r0 + rows, 128 * k:128 * (k + 1)],
                                              dst.at[k * n + r0:k * n + r0 + rows],
                                              sems.at[2 * i + k]) for k in range(2)]
        else:
            self.cps = [pltpu.make_async_copy(src, dst, sems.at[2 * i])]

    def start(self):
        for cp in self.cps:
            cp.start()

    def wait(self):
        for cp in self.cps:
            cp.wait()


def _merge_pair(e, o):
    return jnp.concatenate([e[:, :384], e[:, 384:] + o[:, :128], o[:, 128:]], axis=1)


def _kernel(xa_h, mem0_h, wq_h, wk_h, wv_h, wo_h, xb_h, c_h, wqb_h, wuk_h, wuv_h, wob_h,
            out_h, out_ref, xbt, xb, ckv, wqb, wuk, wuv, wob, wq_s, wk_s, wv_s, sems, *, S, DM, H, DH, MEM, SEG, DC):
    NP = H // 2
    NSEG = S // SEG
    STRIDE = (NSEG - WARM) // NCHAIN
    NPASS = WARM + STRIDE
    scale = DH ** -0.5 * LOG2E
    xb, wq_s, wk_s, wv_s = _as_bf16(xb, wq_s, wk_s, wv_s)

    b_copies = [_Load(s, d, sems, 6 + i) for i, (s, d) in enumerate(
        [(c_h, ckv), (wuk_h, wuk), (wuv_h, wuv), (xb_h, xbt), (wqb_h, wqb), (wob_h, wob)])]

    def branch_a(xat, xa, xs, mem0, me, ms, wo, a_all, b_all, bt_all):
        xa, xs, me, ms, a_all, b_all, bt_all = _as_bf16(xa, xs, me, ms, a_all, b_all, bt_all)

        def precompute(wq, wk, wv, hq, hk):
            hq, hk = _as_bf16(hq, hk)
            x_copy = _Load(xa_h, xat, sems, 0)
            qk_copies = [[_Load(s, d, sems, 12 + 2 * i + k, i * 64 * H, 64 * H)
                          for k, (s, d) in enumerate([(wq_h, wq), (wk_h, wk)])]
                         for i in range(DM // 64)]
            v_copies = [_Load(s, d, sems, 1 + i) for i, (s, d) in enumerate(
                [(wv_h, wv), (wo_h, wo), (mem0_h, mem0)])]
            x_copy.start()
            for cps in qk_copies:
                for cp in cps:
                    cp.start()
            x_copy.wait()

            def make_x(b, _):
                r0 = pl.multiple_of(b * TB, TB)
                xt = xat[:, pl.ds(r0, TB)]
                z = jnp.zeros((64, TB), BF)
                xa[pl.ds(r0, TB), :] = jnp.concatenate([xt, z], axis=0).T
                xs[pl.ds(r0, TB), :] = jnp.concatenate([z, xt], axis=0).T
            lax.fori_loop(0, S // TB, make_x, None)

            for i, cps in enumerate(qk_copies):
                for cp in cps:
                    cp.wait()
                if i == DM // 64 - 2:
                    for cp in v_copies:
                        cp.start()
                _split_heads(wq, hq, i * 64, 64)
                _split_heads(wk, hk, i * 64, 64)

            z = jnp.zeros((64, DH), BF)
            for j in range(NP):
                a0 = _dot_nt(hq[2 * j], jnp.concatenate([hk[2 * j], z], axis=0))
                a1 = _dot_nt(hq[2 * j + 1], jnp.concatenate([z, hk[2 * j + 1]], axis=0))
                a_all[j] = (_merge_pair(a0, a1) * scale).astype(BF)
            for cp in v_copies:
                cp.wait()
            for cp in b_copies:
                cp.start()
            hv = hq
            for i in range(DM // 64):
                _split_heads(wv, hv, i * 64, 64)
            for j in range(NP):
                b0 = _dot_nt(hv[2 * j], jnp.concatenate([wo[2 * j], z], 0)).astype(BF)
                b1 = _dot_nt(hv[2 * j + 1], jnp.concatenate([wo[2 * j + 1], z], 0)).astype(BF)
                b = jnp.concatenate([b0, b1], axis=0)
                b_all[j] = b
                bt_all[j] = b.T[0:DM]

        raw = pltpu.VMEM((2 * DM * H, 128), BF)
        pl.run_scoped(precompute, raw, raw, raw,
                      _packed(H, DM, DH), _packed(H, DM, DH))

        def seg_keys(seg):
            r = pl.ds(pl.multiple_of(seg * SEG, SEG), SEG)
            return (jnp.concatenate([me[seg], xa[r, :]], axis=0),
                    jnp.concatenate([ms[seg], xs[r, :]], axis=0))

        tk = lax.broadcasted_iota(jnp.int32, (48, 128), 0)
        tcol = lax.broadcasted_iota(jnp.int32, (48, 128), 1)
        exists = (tk < MEM) | (tk >= 16)

        def softmax_t(s):
            p = jnp.exp2(s - jnp.max(s, axis=0, keepdims=True))
            return p * (1.0 / jnp.sum(p, axis=0, keepdims=True))

        def one_pass(t, carry):
            mem, spec = carry
            spec = jnp.where(t == WARM, mem, spec)
            sh = pltpu.roll(mem, 64, 1)
            z8 = jnp.zeros((8, 512), F32)
            for c in range(NCHAIN):
                seg = c * STRIDE + t
                me[seg] = jnp.concatenate([mem[8 * c:8 * c + 8], z8], 0).astype(BF)
                ms[seg] = jnp.concatenate([sh[8 * c:8 * c + 8], z8], 0).astype(BF)
            mb = mem[:, :DM].astype(BF)
            qs = [_dot(mb, a_all[j]) for j in range(NP)]
            kcs, ss = [], []
            for c in range(NCHAIN):
                ke, ko = seg_keys(c * STRIDE + t)
                z16 = jnp.zeros((16, 512), BF)
                kcs.append(jnp.concatenate([ke, z16, ko, z16], axis=0))
                lhs = jnp.concatenate(
                    [q[8 * c:8 * c + 8, 0:512] for q in qs]
                    + [q[8 * c:8 * c + 8, 384:896] for q in qs], axis=0).astype(BF)
                ss.append(_dot_nt(kcs[c], lhs))
            even = tcol < 64
            zp = jnp.zeros((16, 128), F32)
            ps = []
            for s in ss:
                p = softmax_t(jnp.where(exists, jnp.where(even, s[0:48], s[64:112]), NEG_PAD))
                ps.append(jnp.concatenate(
                    [jnp.where(even, p, 0.0), zp, jnp.where(even, 0.0, p), zp], 0).T.astype(BF))
            phs = []
            for c in range(NCHAIN):
                r = _dot(ps[c], kcs[c])
                phs.append([_merge_pair(r[8 * j:8 * j + 8], r[64 + 8 * j:72 + 8 * j])
                            for j in range(NP)])
            new = None
            for j in range(NP):
                l = jnp.concatenate([phs[c][j] for c in range(NCHAIN)], axis=0).astype(BF)
                d = _dot(l, b_all[j])
                new = d if new is None else new + d
            return new.astype(BF).astype(F32), spec

        def sweep(state):
            n, _, mem = state
            fin, spec = lax.fori_loop(jnp.where(n == 0, 0, WARM), NPASS, one_pass, (mem, mem))
            nxt = jnp.concatenate([spec[0:8], fin[0:8 * (NCHAIN - 1)]], axis=0)
            diff = pltpu.bitcast(nxt, jnp.int32) != pltpu.bitcast(spec, jnp.int32)
            return n + 1, jnp.max(diff.astype(jnp.int32)), nxt

        m0 = jnp.concatenate([mem0[...].astype(F32), jnp.zeros((MEM, 64), F32)], axis=1)
        lax.while_loop(lambda st: (st[0] < NCHAIN) & (st[1] > 0), sweep,
                       (jnp.int32(0), jnp.int32(1), jnp.concatenate([m0] * NCHAIN, axis=0)))

        visible = (tk < MEM) | ((tk >= 16) & (tk - 16 <= (tcol & (SEG - 1))))
        fill = jnp.where(exists, NEG_MASK, NEG_PAD).astype(F32)

        def probs_t(s):
            return softmax_t(jnp.where(visible, s, fill))

        for cp in b_copies:
            cp.wait()

        def tokens(qp, ph):
            qp, ph = _as_bf16(qp, ph)

            def tok_block(b, _):
                def project(u, j):
                    x = xa[pl.ds(pl.multiple_of((2 * b + u) * TB, TB), TB), 0:DM]
                    d = _dot(x, a_all[j])
                    qp[u, j] = d.astype(BF)
                    return [d[24 * (k % 5):24 * (k % 5) + 8, 768 * (k // 5):768 * (k // 5) + 128]
                            for k in range(10)]

                def scores(u, g):
                    ke, ko = seg_keys((2 * b + u) * (TB // SEG) + g)
                    rows = slice(g * SEG, (g + 1) * SEG)
                    res = []
                    for j0 in range(0, NP, 4):
                        js = range(j0, j0 + 4)
                        res.append((
                            _dot_nt(ke, jnp.concatenate([qp[u, j, rows, 0:512] for j in js], 0)),
                            _dot_nt(ko, jnp.concatenate([qp[u, j, rows, 384:896] for j in js], 0))))
                    return res

                def probs(sc):
                    zp = jnp.zeros((16, 128), F32)
                    return [jnp.concatenate([probs_t(se), zp, probs_t(so), zp], 0).T.astype(BF)
                            for se, so in sc]

                def mix(u, g, ps):
                    ke, ko = seg_keys((2 * b + u) * (TB // SEG) + g)
                    z = jnp.zeros((48, 384), BF)
                    z16 = jnp.zeros((16, 2 * DM), BF)
                    kc = jnp.concatenate([jnp.concatenate([ke, z], axis=1), z16,
                                          jnp.concatenate([z, ko], axis=1), z16], axis=0)
                    r = _dot(jnp.concatenate(ps, axis=0), kc).astype(BF)
                    for j in range(NP):
                        ph[u, j, g * SEG:(g + 1) * SEG, :] = r[SEG * j:SEG * (j + 1)]

                def side(j, after):
                    m0 = pl.multiple_of(b * 128 + j * 16, 16)
                    _split_heads(wuk, wk_s, m0, 16, after)
                    _split_heads(wuv, wv_s, m0, 16, after)
                    mq = jnp.minimum(b, DM // 64 - 1) * 64 + j // 2 * 16
                    _split_heads(wqb, wq_s, pl.multiple_of(mq, 16), 16, after, (j % 2,))

                def emit(u, acc):
                    r = pl.ds(pl.multiple_of((2 * b + u) * TB, TB), TB)
                    z = jnp.zeros((64, TB), BF)
                    out_ref[r, 0:512] = jnp.concatenate([acc.astype(BF), z], axis=0).T
                    xb[r, :] = jnp.concatenate([xbt[:, r], z], axis=0).T

                for j in range(NP):
                    side(j, project(0, j))
                for g in range(TB // SEG):
                    sc = scores(0, g)
                    project(1, 2 * g)
                    project(1, 2 * g + 1)
                    mix(0, g, probs(sc))
                acc = None
                for g in range(TB // SEG):
                    sc = scores(1, g)
                    for j in (2 * g, 2 * g + 1):
                        d = _dot_nt(bt_all[j], ph[0, j])
                        acc = d if acc is None else acc + d
                    mix(1, g, probs(sc))
                emit(0, acc)
                acc = None
                for j in range(NP):
                    d = _dot_nt(bt_all[j], ph[1, j])
                    acc = d if acc is None else acc + d
                emit(1, acc)
            lax.fori_loop(0, S // (2 * TB), tok_block, None)

        pl.run_scoped(tokens, _packed(2, NP, TB, 2 * DM), _packed(2, NP, TB, 2 * DM))

    pl.run_scoped(
        branch_a,
        pltpu.VMEM((DM, S), BF), _packed(S, 512), _packed(S, 512),
        pltpu.VMEM((MEM, DM), BF),
        _packed(NSEG, 16, 512), _packed(NSEG, 16, 512),
        pltpu.VMEM((H, DM, DH), BF),
        _packed(NP, DM, 2 * DM), _packed(NP, 2 * DM, 512),
        _packed(NP, DM, 2 * DM))

    def branch_b(ctx, q_s, k_s, v_s, cs):
        ctx, q_s, k_s, v_s, cs = _as_bf16(ctx, q_s, k_s, v_s, cs)
        qi = lax.broadcasted_iota(jnp.int32, (QB, QB // 2), 0)
        kj = lax.broadcasted_iota(jnp.int32, (QB, QB // 2), 1)
        causal = kj <= qi

        S2, C2, D2 = S // 2, DC // 2, DH // 2

        def add(x, y, sign=1):
            return (x.astype(F32) + sign * y.astype(F32)).astype(BF)

        def latent_sums(i, _):
            r = pl.ds(pl.multiple_of(i * 128, 128), 128)
            r2 = pl.ds(pl.multiple_of(S2 + i * 128, 128), 128)
            a11, a12, a21, a22 = ckv[r, 0:C2], ckv[r, C2:DC], ckv[r2, 0:C2], ckv[r2, C2:DC]
            cs[0, r, :] = add(a11, a22)
            cs[1, r, :] = add(a21, a22)
            cs[2, r, :] = add(a11, a12)
            cs[3, r, :] = add(a21, a11, -1)
            cs[4, r, :] = add(a12, a22, -1)
        lax.fori_loop(0, S2 // 128, latent_sums, None)

        def project_kv(h):
            def quad(i, j):
                r, c = slice(i * C2, (i + 1) * C2), slice(j * D2, (j + 1) * D2)
                return jnp.concatenate([wk_s[h, r, c], wv_s[h, r, c]], axis=1)

            def put(i, j, val):
                r, c = slice(i * S2, (i + 1) * S2), slice(j * D2, (j + 1) * D2)
                k_s[r, c] = val[:, 0:D2].astype(BF)
                v_s[r, c] = val[:, D2:DH].astype(BF)

            b11, b12, b21, b22 = quad(0, 0), quad(0, 1), quad(1, 0), quad(1, 1)
            m2 = _dot(cs[1], b11)
            m4 = _dot(ckv[S2:S, C2:DC], add(b21, b11, -1))
            put(1, 0, m2 + m4)
            m5 = _dot(cs[2], b22)
            m3 = _dot(ckv[0:S2, 0:C2], add(b12, b22, -1))
            put(0, 1, m3 + m5)
            m1 = _dot(cs[0], add(b11, b22))
            put(0, 0, (m4 - m5) + m1 + _dot(cs[4], add(b21, b22)))
            put(1, 1, (m3 - m2) + m1 + _dot(cs[3], add(b11, b12)))

        def head(h, _):
            q_s[...] = (_dot(xb[:, 0:DM], wq_s[h]) * scale).astype(BF)
            project_kv(h)

            def scores(i):
                lo, mid, hi = i * QB, i * QB + QB // 2, (i + 1) * QB
                q = q_s[lo:hi, :]
                return (_dot_nt(q, k_s[0:mid, :]), _dot_nt(q[QB // 2:], k_s[mid:hi, :]))

            def attend(i, sa, sb):
                lo, mid, hi = i * QB, i * QB + QB // 2, (i + 1) * QB
                cols = [sa[:, c:c + 128] for c in range(0, mid, 128)]
                cols[-1] = jnp.where(causal, cols[-1], NEG_MASK)
                sb = jnp.where(causal[0:QB // 2], sb, NEG_MASK)
                m = functools.reduce(jnp.maximum, cols)
                m = jnp.concatenate([m[:QB // 2], jnp.maximum(m[QB // 2:], sb)], axis=0)
                m = jnp.max(m, axis=-1, keepdims=True)
                cols = [jnp.exp2(c - m) for c in cols]
                pb = jnp.exp2(sb - m[QB // 2:])
                l = functools.reduce(jnp.add, cols)
                l = jnp.concatenate([l[:QB // 2], l[QB // 2:] + pb], axis=0)
                l = jnp.sum(l, axis=-1, keepdims=True)
                o = _dot(jnp.concatenate(cols, axis=1).astype(BF), v_s[0:mid, :])
                ob = _dot(pb.astype(BF), v_s[mid:hi, :])
                o = jnp.concatenate([o[:QB // 2], o[QB // 2:] + ob], axis=0)
                ctx[h, lo:hi, :] = (o * (1.0 / l)).astype(BF)

            nxt = scores(S // QB - 1)
            for i in reversed(range(S // QB)):
                cur = nxt
                if i:
                    nxt = scores(i - 1)
                attend(i, *cur)
        lax.fori_loop(0, H, head, None)

        lane = lax.broadcasted_iota(jnp.int32, (512, 128), 1)

        def store(i):
            r = pl.ds(pl.multiple_of(i * 512, 512), 512)
            return pltpu.make_async_copy(out_ref.at[r], out_h.at[r], sems.at[52 + i])

        def out_block(i, _):
            r = pl.ds(pl.multiple_of(i * 512, 512), 512)
            acc = None
            for h in range(H):
                d = _dot_nt(wob[h], ctx[h, r, :])
                acc = d if acc is None else acc + d
            res = jnp.concatenate([jnp.zeros((64, 512), BF), acc.astype(BF)], axis=0).T
            out_ref[r, 384:512] = jnp.where(lane < 64, out_ref[r, 384:512], res[:, 0:128])
            out_ref[r, 512:896] = res[:, 128:512]
            store(i).start()
        lax.fori_loop(0, S // 512, out_block, None)
        for i in range(S // 512):
            store(i).wait()

    pl.run_scoped(
        branch_b,
        _packed(H, S, DH),
        _packed(S, DH), _packed(S, DH), _packed(S, DH), _packed(5, S // 2, DC // 2))


@functools.partial(jax.jit, static_argnames=("A_seg_len",))
def pallas_concat_heads__memory_aug_recurrent_mem_tr__compressed_kv_cla__prompt_kernel(
    A_x, A_mem0, A_Wq, A_Wk, A_Wv, A_Wo, A_seg_len,
    B_x, B_c_kv, B_w_q, B_w_uk, B_w_uv, B_w_o,
):
    _, S, DM = A_x.shape
    _, H, DH = A_Wq.shape
    MEM = A_mem0.shape[1]
    DC = B_c_kv.shape[2]
    assert (S, DM, H, DH, MEM, A_seg_len, DC) == (2048, 448, 16, 256, 8, 32, 1024)
    assert B_x.shape == A_x.shape and B_c_kv.shape[1] == S

    out = pl.pallas_call(
        functools.partial(_kernel, S=S, DM=DM, H=H, DH=DH, MEM=MEM, SEG=A_seg_len, DC=DC),
        out_shape=jax.ShapeDtypeStruct((S, 2 * DM), BF),
        in_specs=[pl.BlockSpec(memory_space=pl.ANY)] * 12,
        out_specs=pl.BlockSpec(memory_space=pl.ANY),
        scratch_shapes=[
            pltpu.VMEM((S, 2 * DM), BF),
            pltpu.VMEM((DM, S), BF), _packed(S, 512), pltpu.VMEM((S, DC), BF),
            pltpu.VMEM((2 * DM * H, 128), BF), pltpu.VMEM((2 * DC * H, 128), BF),
            pltpu.VMEM((2 * DC * H, 128), BF), pltpu.VMEM((H, DM, DH), BF),
            _packed(H, DM, DH), _packed(H, DC, DH), _packed(H, DC, DH),
            pltpu.SemaphoreType.DMA((56,)),
        ],
        compiler_params=pltpu.CompilerParams(vmem_limit_bytes=120 * 1024 * 1024),
    )(
        A_x.reshape(S, DM).T, A_mem0.reshape(MEM, DM),
        A_Wq.reshape(DM * H, DH), A_Wk.reshape(DM * H, DH), A_Wv.reshape(DM * H, DH),
        A_Wo.transpose(0, 2, 1),
        B_x.reshape(S, DM).T, B_c_kv.reshape(S, DC),
        B_w_q.reshape(DM * H, DH), B_w_uk.reshape(DC * H, DH), B_w_uv.reshape(DC * H, DH),
        B_w_o.transpose(0, 2, 1),
    )
    return out.reshape(1, S, 2 * DM)
```

```python
import functools
import math

import jax
import jax.numpy as jnp
from jax import lax
import jax.experimental.pallas as pl
import jax.experimental.pallas.tpu as pltpu

BF = jnp.bfloat16
F32 = jnp.float32
LOG2E = math.log2(math.e)
NEG_MASK = -1e9 * LOG2E
NEG_PAD = -3e38

NCHAIN = 4
WARM = 4
TB = 128
QB = 256


def _dot(a, b):
    return jnp.dot(a, b, preferred_element_type=F32)


def _dot_nt(a, b):
    return lax.dot_general(a, b, (((1,), (1,)), ((), ())), preferred_element_type=F32)


def _split_heads(raw_ref, dst_ref, m0, rows, after=None, halves=(0, 1)):
    u = raw_ref.bitcast(jnp.uint32)
    half = u.shape[0] // 2
    g = rows // 8
    sub = lax.broadcasted_iota(jnp.int32, (g, 8, 128), 1)
    for i in halves:
        w = u[pl.ds(pl.multiple_of(i * half + m0 * 8, 64), rows * 8), :].reshape(g, 8, 8, 128)
        if after is not None:
            pins = jnp.stack([after.pop(0) for _ in range(g)])[:, None]
            w = w | ((pltpu.bitcast(pins, jnp.uint32) >> 31) >> 1)
        v = [w[:, m] for m in range(8)]
        for d in (4, 2, 1):
            keep = (sub & d) == 0
            for a in range(8):
                if not a & d:
                    x, y = v[a], v[a + d]
                    v[a] = jnp.where(keep, x, pltpu.roll(y, d, 1))
                    v[a + d] = jnp.where(keep, pltpu.roll(x, 8 - d, 1), y)
        for p in range(8):
            x = v[p].reshape(rows, 128)
            lo = pltpu.bitcast(x << 16, F32).astype(BF)
            hi = pltpu.bitcast(x & jnp.uint32(0xFFFF0000), F32).astype(BF)
            dst_ref[2 * p, pl.ds(m0, rows), 128 * i:128 * (i + 1)] = lo
            dst_ref[2 * p + 1, pl.ds(m0, rows), 128 * i:128 * (i + 1)] = hi


def _packed(*shape):
    return pltpu.VMEM(shape[:-2] + (shape[-2] // 2, shape[-1]), jnp.uint32)


def _as_bf16(*refs):
    return [r.bitcast(BF) for r in refs]


class _Load:
    def __init__(self, src, dst, sems, i, r0=0, rows=None):
        n = src.shape[0]
        rows = rows or n
        if dst.shape != src.shape:
            self.cps = [pltpu.make_async_copy(src.at[r0:r0 + rows, 128 * k:128 * (k + 1)],
                                              dst.at[k * n + r0:k * n + r0 + rows],
                                              sems.at[2 * i + k]) for k in range(2)]
        else:
            self.cps = [pltpu.make_async_copy(src, dst, sems.at[2 * i])]

    def start(self):
        for cp in self.cps:
            cp.start()

    def wait(self):
        for cp in self.cps:
            cp.wait()


def _merge_pair(e, o):
    return jnp.concatenate([e[:, :384], e[:, 384:] + o[:, :128], o[:, 128:]], axis=1)


def _kernel(xa_h, mem0_h, wq_h, wk_h, wv_h, wo_h, xb_h, c_h, wqb_h, wuk_h, wuv_h, wob_h,
            out_h, out_ref, xbt, xb, ckv, wqb, wuk, wuv, wob, wq_s, wk_s, wv_s, sems, *, S, DM, H, DH, MEM, SEG, DC):
    NP = H // 2
    NSEG = S // SEG
    STRIDE = (NSEG - WARM) // NCHAIN
    NPASS = WARM + STRIDE
    scale = DH ** -0.5 * LOG2E
    xb, wq_s, wk_s, wv_s = _as_bf16(xb, wq_s, wk_s, wv_s)

    b_copies = [_Load(s, d, sems, 6 + i) for i, (s, d) in enumerate(
        [(c_h, ckv), (wuk_h, wuk), (wuv_h, wuv), (xb_h, xbt), (wqb_h, wqb), (wob_h, wob)])]

    def branch_a(xat, xa, xs, mem0, me, ms, wo, a_all, b_all, bt_all):
        xa, xs, me, ms, a_all, b_all, bt_all = _as_bf16(xa, xs, me, ms, a_all, b_all, bt_all)

        def precompute(wq, wk, wv, hq, hk):
            hq, hk = _as_bf16(hq, hk)
            x_copy = _Load(xa_h, xat, sems, 0)
            qk_copies = [[_Load(s, d, sems, 12 + 2 * i + k, i * 64 * H, 64 * H)
                          for k, (s, d) in enumerate([(wq_h, wq), (wk_h, wk)])]
                         for i in range(DM // 64)]
            v_copies = [_Load(s, d, sems, 1 + i) for i, (s, d) in enumerate(
                [(wv_h, wv), (wo_h, wo), (mem0_h, mem0)])]
            x_copy.start()
            for cps in qk_copies:
                for cp in cps:
                    cp.start()
            x_copy.wait()

            def make_x(b, _):
                r0 = pl.multiple_of(b * TB, TB)
                xt = xat[:, pl.ds(r0, TB)]
                z = jnp.zeros((64, TB), BF)
                xa[pl.ds(r0, TB), :] = jnp.concatenate([xt, z], axis=0).T
                xs[pl.ds(r0, TB), :] = jnp.concatenate([z, xt], axis=0).T
            lax.fori_loop(0, S // TB, make_x, None)

            for i, cps in enumerate(qk_copies):
                for cp in cps:
                    cp.wait()
                if i == DM // 64 - 2:
                    for cp in v_copies:
                        cp.start()
                _split_heads(wq, hq, i * 64, 64)
                _split_heads(wk, hk, i * 64, 64)

            z = jnp.zeros((64, DH), BF)
            for j in range(NP):
                a0 = _dot_nt(hq[2 * j], jnp.concatenate([hk[2 * j], z], axis=0))
                a1 = _dot_nt(hq[2 * j + 1], jnp.concatenate([z, hk[2 * j + 1]], axis=0))
                a_all[j] = (_merge_pair(a0, a1) * scale).astype(BF)
            for cp in v_copies:
                cp.wait()
            for cp in b_copies:
                cp.start()
            hv = hq
            for i in range(DM // 64):
                _split_heads(wv, hv, i * 64, 64)
            for j in range(NP):
                b0 = _dot_nt(hv[2 * j], jnp.concatenate([wo[2 * j], z], 0)).astype(BF)
                b1 = _dot_nt(hv[2 * j + 1], jnp.concatenate([wo[2 * j + 1], z], 0)).astype(BF)
                b = jnp.concatenate([b0, b1], axis=0)
                b_all[j] = b
                bt_all[j] = b.T[0:DM]

        raw = pltpu.VMEM((2 * DM * H, 128), BF)
        pl.run_scoped(precompute, raw, raw, raw,
                      _packed(H, DM, DH), _packed(H, DM, DH))

        def seg_keys(seg):
            r = pl.ds(pl.multiple_of(seg * SEG, SEG), SEG)
            return (jnp.concatenate([me[seg], xa[r, :]], axis=0),
                    jnp.concatenate([ms[seg], xs[r, :]], axis=0))

        tk = lax.broadcasted_iota(jnp.int32, (48, 128), 0)
        tcol = lax.broadcasted_iota(jnp.int32, (48, 128), 1)
        exists = (tk < MEM) | (tk >= 16)

        def softmax_t(s):
            p = jnp.exp2(s - jnp.max(s, axis=0, keepdims=True))
            return p * (1.0 / jnp.sum(p, axis=0, keepdims=True))

        def one_pass(t, carry):
            mem, spec = carry
            spec = jnp.where(t == WARM, mem, spec)
            sh = pltpu.roll(mem, 64, 1)
            z8 = jnp.zeros((8, 512), F32)
            for c in range(NCHAIN):
                seg = c * STRIDE + t
                me[seg] = jnp.concatenate([mem[8 * c:8 * c + 8], z8], 0).astype(BF)
                ms[seg] = jnp.concatenate([sh[8 * c:8 * c + 8], z8], 0).astype(BF)
            mb = mem[:, :DM].astype(BF)
            qs = [_dot(mb, a_all[j]) for j in range(NP)]
            kcs, ss = [], []
            for c in range(NCHAIN):
                ke, ko = seg_keys(c * STRIDE + t)
                z16 = jnp.zeros((16, 512), BF)
                kcs.append(jnp.concatenate([ke, z16, ko, z16], axis=0))
                lhs = jnp.concatenate(
                    [q[8 * c:8 * c + 8, 0:512] for q in qs]
                    + [q[8 * c:8 * c + 8, 384:896] for q in qs], axis=0).astype(BF)
                ss.append(_dot_nt(kcs[c], lhs))
            even = tcol < 64
            zp = jnp.zeros((16, 128), F32)
            ps = []
            for s in ss:
                p = softmax_t(jnp.where(exists, jnp.where(even, s[0:48], s[64:112]), NEG_PAD))
                ps.append(jnp.concatenate(
                    [jnp.where(even, p, 0.0), zp, jnp.where(even, 0.0, p), zp], 0).T.astype(BF))
            phs = []
            for c in range(NCHAIN):
                r = _dot(ps[c], kcs[c])
                phs.append([_merge_pair(r[8 * j:8 * j + 8], r[64 + 8 * j:72 + 8 * j])
                            for j in range(NP)])
            new = None
            for j in range(NP):
                l = jnp.concatenate([phs[c][j] for c in range(NCHAIN)], axis=0).astype(BF)
                d = _dot(l, b_all[j])
                new = d if new is None else new + d
            return new.astype(BF).astype(F32), spec

        def sweep(state):
            n, _, mem = state
            fin, spec = lax.fori_loop(jnp.where(n == 0, 0, WARM), NPASS, one_pass, (mem, mem))
            nxt = jnp.concatenate([spec[0:8], fin[0:8 * (NCHAIN - 1)]], axis=0)
            diff = pltpu.bitcast(nxt, jnp.int32) != pltpu.bitcast(spec, jnp.int32)
            return n + 1, jnp.max(diff.astype(jnp.int32)), nxt

        m0 = jnp.concatenate([mem0[...].astype(F32), jnp.zeros((MEM, 64), F32)], axis=1)
        lax.while_loop(lambda st: (st[0] < NCHAIN) & (st[1] > 0), sweep,
                       (jnp.int32(0), jnp.int32(1), jnp.concatenate([m0] * NCHAIN, axis=0)))

        visible = (tk < MEM) | ((tk >= 16) & (tk - 16 <= (tcol & (SEG - 1))))
        fill = jnp.where(exists, NEG_MASK, NEG_PAD).astype(F32)

        def probs_t(s):
            return softmax_t(jnp.where(visible, s, fill))

        for cp in b_copies:
            cp.wait()

        def tokens(qp, ph):
            qp, ph = _as_bf16(qp, ph)

            def tok_block(b, _):
                def project(u, j):
                    x = xa[pl.ds(pl.multiple_of((2 * b + u) * TB, TB), TB), 0:DM]
                    d = _dot(x, a_all[j])
                    qp[u, j] = d.astype(BF)
                    return [d[24 * (k % 5):24 * (k % 5) + 8, 768 * (k // 5):768 * (k // 5) + 128]
                            for k in range(10)]

                def scores(u, g):
                    ke, ko = seg_keys((2 * b + u) * (TB // SEG) + g)
                    rows = slice(g * SEG, (g + 1) * SEG)
                    res = []
                    for j0 in range(0, NP, 4):
                        js = range(j0, j0 + 4)
                        res.append((
                            _dot_nt(ke, jnp.concatenate([qp[u, j, rows, 0:512] for j in js], 0)),
                            _dot_nt(ko, jnp.concatenate([qp[u, j, rows, 384:896] for j in js], 0))))
                    return res

                def probs(sc):
                    zp = jnp.zeros((16, 128), F32)
                    return [jnp.concatenate([probs_t(se), zp, probs_t(so), zp], 0).T.astype(BF)
                            for se, so in sc]

                def mix(u, g, ps):
                    ke, ko = seg_keys((2 * b + u) * (TB // SEG) + g)
                    z = jnp.zeros((48, 384), BF)
                    z16 = jnp.zeros((16, 2 * DM), BF)
                    kc = jnp.concatenate([jnp.concatenate([ke, z], axis=1), z16,
                                          jnp.concatenate([z, ko], axis=1), z16], axis=0)
                    r = _dot(jnp.concatenate(ps, axis=0), kc).astype(BF)
                    for j in range(NP):
                        ph[u, j, g * SEG:(g + 1) * SEG, :] = r[SEG * j:SEG * (j + 1)]

                def side(j, after):
                    m0 = pl.multiple_of(b * 128 + j * 16, 16)
                    _split_heads(wuk, wk_s, m0, 16, after)
                    _split_heads(wuv, wv_s, m0, 16, after)
                    mq = jnp.minimum(b, DM // 64 - 1) * 64 + j // 2 * 16
                    _split_heads(wqb, wq_s, pl.multiple_of(mq, 16), 16, after, (j % 2,))

                def emit(u, acc):
                    r = pl.ds(pl.multiple_of((2 * b + u) * TB, TB), TB)
                    z = jnp.zeros((64, TB), BF)
                    out_ref[r, 0:512] = jnp.concatenate([acc.astype(BF), z], axis=0).T
                    xb[r, :] = jnp.concatenate([xbt[:, r], z], axis=0).T

                for j in range(NP):
                    side(j, project(0, j))
                for g in range(TB // SEG):
                    sc = scores(0, g)
                    project(1, 2 * g)
                    project(1, 2 * g + 1)
                    mix(0, g, probs(sc))
                acc = None
                for g in range(TB // SEG):
                    sc = scores(1, g)
                    for j in (2 * g, 2 * g + 1):
                        d = _dot_nt(bt_all[j], ph[0, j])
                        acc = d if acc is None else acc + d
                    mix(1, g, probs(sc))
                emit(0, acc)
                acc = None
                for j in range(NP):
                    d = _dot_nt(bt_all[j], ph[1, j])
                    acc = d if acc is None else acc + d
                emit(1, acc)
            lax.fori_loop(0, S // (2 * TB), tok_block, None)

        pl.run_scoped(tokens, _packed(2, NP, TB, 2 * DM), _packed(2, NP, TB, 2 * DM))

    pl.run_scoped(
        branch_a,
        pltpu.VMEM((DM, S), BF), _packed(S, 512), _packed(S, 512),
        pltpu.VMEM((MEM, DM), BF),
        _packed(NSEG, 16, 512), _packed(NSEG, 16, 512),
        pltpu.VMEM((H, DM, DH), BF),
        _packed(NP, DM, 2 * DM), _packed(NP, 2 * DM, 512),
        _packed(NP, DM, 2 * DM))

    def branch_b(ctx, slot, k_s, v_s, cs):
        ctx, k_s, v_s, cs = _as_bf16(ctx, k_s, v_s, cs)
        qi = lax.broadcasted_iota(jnp.int32, (QB, QB // 2), 0)
        kj = lax.broadcasted_iota(jnp.int32, (QB, QB // 2), 1)
        causal = kj <= qi

        S2, C2, D2 = S // 2, DC // 2, DH // 2

        def add(x, y, sign=1):
            return (x.astype(F32) + sign * y.astype(F32)).astype(BF)

        def latent_sums(i, _):
            r = pl.ds(pl.multiple_of(i * 128, 128), 128)
            r2 = pl.ds(pl.multiple_of(S2 + i * 128, 128), 128)
            a11, a12, a21, a22 = ckv[r, 0:C2], ckv[r, C2:DC], ckv[r2, 0:C2], ckv[r2, C2:DC]
            cs[0, r, :] = add(a11, a22)
            cs[1, r, :] = add(a21, a22)
            cs[2, r, :] = add(a11, a12)
            cs[3, r, :] = add(a21, a11, -1)
            cs[4, r, :] = add(a12, a22, -1)
        lax.fori_loop(0, S2 // 128, latent_sums, None)

        def project_kv(h):
            def quad(i, j):
                r, c = slice(i * C2, (i + 1) * C2), slice(j * D2, (j + 1) * D2)
                return jnp.concatenate([wk_s[h, r, c], wv_s[h, r, c]], axis=1)

            def put(i, j, val):
                r, c = slice(i * S2, (i + 1) * S2), slice(j * D2, (j + 1) * D2)
                k_s[r, c] = val[:, 0:D2].astype(BF)
                v_s[r, c] = val[:, D2:DH].astype(BF)

            b11, b12, b21, b22 = quad(0, 0), quad(0, 1), quad(1, 0), quad(1, 1)
            m2 = _dot(cs[1], b11)
            m4 = _dot(ckv[S2:S, C2:DC], add(b21, b11, -1))
            put(1, 0, m2 + m4)
            m5 = _dot(cs[2], b22)
            m3 = _dot(ckv[0:S2, 0:C2], add(b12, b22, -1))
            put(0, 1, m3 + m5)
            m1 = _dot(cs[0], add(b11, b22))
            put(0, 0, (m4 - m5) + m1 + _dot(cs[4], add(b21, b22)))
            put(1, 1, (m3 - m2) + m1 + _dot(cs[3], add(b11, b12)))

        def head(h, _):
            slot[h] = h
            hq = slot[h]
            ctx[hq] = (_dot(xb[:, 0:DM], wq_s[h]) * scale).astype(BF)
            project_kv(h)

            def scores(i):
                lo, mid, hi = i * QB, i * QB + QB // 2, (i + 1) * QB
                q = ctx[hq, lo:hi, :]
                return (_dot_nt(q, k_s[0:mid, :]), _dot_nt(q[QB // 2:], k_s[mid:hi, :]))

            def attend(i, sa, sb):
                lo, mid, hi = i * QB, i * QB + QB // 2, (i + 1) * QB
                cols = [sa[:, c:c + 128] for c in range(0, mid, 128)]
                cols[-1] = jnp.where(causal, cols[-1], NEG_MASK)
                sb = jnp.where(causal[0:QB // 2], sb, NEG_MASK)
                m = functools.reduce(jnp.maximum, cols)
                m = jnp.concatenate([m[:QB // 2], jnp.maximum(m[QB // 2:], sb)], axis=0)
                m = jnp.max(m, axis=-1, keepdims=True)
                cols = [jnp.exp2(c - m) for c in cols]
                pb = jnp.exp2(sb - m[QB // 2:])
                l = functools.reduce(jnp.add, cols)
                l = jnp.concatenate([l[:QB // 2], l[QB // 2:] + pb], axis=0)
                l = jnp.sum(l, axis=-1, keepdims=True)
                o = _dot(jnp.concatenate(cols, axis=1).astype(BF), v_s[0:mid, :])
                ob = _dot(pb.astype(BF), v_s[mid:hi, :])
                o = jnp.concatenate([o[:QB // 2], o[QB // 2:] + ob], axis=0)
                return (o * (1.0 / l)).astype(BF)

            nxt = scores(S // QB - 1)
            for i in reversed(range(S // QB)):
                cur = nxt
                if i:
                    nxt = scores(i - 1)
                if i < S // QB - 1:
                    ctx[h, (i + 1) * QB:(i + 2) * QB, :] = done
                done = attend(i, *cur)
            ctx[h, 0:QB, :] = done
        lax.fori_loop(0, H, head, None)

        lane = lax.broadcasted_iota(jnp.int32, (512, 128), 1)

        def store(i):
            r = pl.ds(pl.multiple_of(i * 512, 512), 512)
            return pltpu.make_async_copy(out_ref.at[r], out_h.at[r], sems.at[52 + i])

        def out_block(i, _):
            r = pl.ds(pl.multiple_of(i * 512, 512), 512)
            acc = None
            for h in range(H):
                d = _dot_nt(wob[h], ctx[h, r, :])
                acc = d if acc is None else acc + d
            res = jnp.concatenate([jnp.zeros((64, 512), BF), acc.astype(BF)], axis=0).T
            out_ref[r, 384:512] = jnp.where(lane < 64, out_ref[r, 384:512], res[:, 0:128])
            out_ref[r, 512:896] = res[:, 128:512]
            store(i).start()
        lax.fori_loop(0, S // 512, out_block, None)
        for i in range(S // 512):
            store(i).wait()

    pl.run_scoped(
        branch_b,
        _packed(H, S, DH), pltpu.SMEM((H,), jnp.int32),
        _packed(S, DH), _packed(S, DH), _packed(5, S // 2, DC // 2))


@functools.partial(jax.jit, static_argnames=("A_seg_len",))
def pallas_concat_heads__memory_aug_recurrent_mem_tr__compressed_kv_cla__prompt_kernel(
    A_x, A_mem0, A_Wq, A_Wk, A_Wv, A_Wo, A_seg_len,
    B_x, B_c_kv, B_w_q, B_w_uk, B_w_uv, B_w_o,
):
    _, S, DM = A_x.shape
    _, H, DH = A_Wq.shape
    MEM = A_mem0.shape[1]
    DC = B_c_kv.shape[2]
    assert (S, DM, H, DH, MEM, A_seg_len, DC) == (2048, 448, 16, 256, 8, 32, 1024)
    assert B_x.shape == A_x.shape and B_c_kv.shape[1] == S

    out = pl.pallas_call(
        functools.partial(_kernel, S=S, DM=DM, H=H, DH=DH, MEM=MEM, SEG=A_seg_len, DC=DC),
        out_shape=jax.ShapeDtypeStruct((S, 2 * DM), BF),
        in_specs=[pl.BlockSpec(memory_space=pl.ANY)] * 12,
        out_specs=pl.BlockSpec(memory_space=pl.ANY),
        scratch_shapes=[
            pltpu.VMEM((S, 2 * DM), BF),
            pltpu.VMEM((DM, S), BF), _packed(S, 512), pltpu.VMEM((S, DC), BF),
            pltpu.VMEM((2 * DM * H, 128), BF), pltpu.VMEM((2 * DC * H, 128), BF),
            pltpu.VMEM((2 * DC * H, 128), BF), pltpu.VMEM((H, DM, DH), BF),
            _packed(H, DM, DH), _packed(H, DC, DH), _packed(H, DC, DH),
            pltpu.SemaphoreType.DMA((56,)),
        ],
        compiler_params=pltpu.CompilerParams(vmem_limit_bytes=120 * 1024 * 1024),
    )(
        A_x.reshape(S, DM).T, A_mem0.reshape(MEM, DM),
        A_Wq.reshape(DM * H, DH), A_Wk.reshape(DM * H, DH), A_Wv.reshape(DM * H, DH),
        A_Wo.transpose(0, 2, 1),
        B_x.reshape(S, DM).T, B_c_kv.reshape(S, DC),
        B_w_q.reshape(DM * H, DH), B_w_uk.reshape(DC * H, DH), B_w_uv.reshape(DC * H, DH),
        B_w_o.transpose(0, 2, 1),
    )
    return out.reshape(1, S, 2 * DM)
```

```python
import functools
import math

import jax
import jax.numpy as jnp
from jax import lax
import jax.experimental.pallas as pl
import jax.experimental.pallas.tpu as pltpu

BF = jnp.bfloat16
F32 = jnp.float32
LOG2E = math.log2(math.e)
NEG_MASK = -1e9 * LOG2E
NEG_PAD = -3e38

NCHAIN = 4
WARM = 4
TB = 128
QB = 256


def _dot(a, b):
    return jnp.dot(a, b, preferred_element_type=F32)


def _dot_nt(a, b):
    return lax.dot_general(a, b, (((1,), (1,)), ((), ())), preferred_element_type=F32)


def _split_heads(raw_ref, dst_ref, m0, rows, after=None, halves=(0, 1)):
    half = raw_ref.shape[0] // 2
    g = rows // 8
    sub = lax.broadcasted_iota(jnp.int32, (g, 8, 128), 1)
    for i in halves:
        w = raw_ref[pl.ds(pl.multiple_of(i * half + m0 * 16, 128), rows * 16), :]
        w = pltpu.bitcast(w, jnp.uint32).reshape(g, 8, 8, 128)
        if after is not None:
            pins = jnp.stack([after.pop(0) for _ in range(g)])[:, None]
            w = w | ((pltpu.bitcast(pins, jnp.uint32) >> 31) >> 1)
        v = [w[:, m] for m in range(8)]
        for d in (4, 2, 1):
            keep = (sub & d) == 0
            for a in range(8):
                if not a & d:
                    x, y = v[a], v[a + d]
                    v[a] = jnp.where(keep, x, pltpu.roll(y, d, 1))
                    v[a + d] = jnp.where(keep, pltpu.roll(x, 8 - d, 1), y)
        for p in range(8):
            x = v[p].reshape(rows, 128)
            lo = pltpu.bitcast(x << 16, F32).astype(BF)
            hi = pltpu.bitcast(x & jnp.uint32(0xFFFF0000), F32).astype(BF)
            dst_ref[2 * p, pl.ds(m0, rows), 128 * i:128 * (i + 1)] = lo
            dst_ref[2 * p + 1, pl.ds(m0, rows), 128 * i:128 * (i + 1)] = hi


def _packed(*shape):
    return pltpu.VMEM(shape[:-2] + (shape[-2] // 2, shape[-1]), jnp.uint32)


def _as_bf16(*refs):
    return [r.bitcast(BF) for r in refs]


class _Load:
    def __init__(self, src, dst, sems, i, r0=0, rows=None):
        n = src.shape[0]
        rows = rows or n
        if dst.shape != src.shape:
            self.cps = [pltpu.make_async_copy(src.at[r0:r0 + rows, 128 * k:128 * (k + 1)],
                                              dst.at[k * n + r0:k * n + r0 + rows],
                                              sems.at[2 * i + k]) for k in range(2)]
        else:
            self.cps = [pltpu.make_async_copy(src, dst, sems.at[2 * i])]

    def start(self):
        for cp in self.cps:
            cp.start()

    def wait(self):
        for cp in self.cps:
            cp.wait()


def _add(x, y, sign=1):
    x, y = x.astype(F32), y.astype(F32)
    return (x + y if sign > 0 else x - y).astype(BF)


def _merge_pair(e, o):
    return jnp.concatenate([e[:, :384], e[:, 384:] + o[:, :128], o[:, 128:]], axis=1)


def _kernel(xa_h, mem0_h, wq_h, wk_h, wv_h, wo_h, xb_h, c_h, wqb_h, wuk_h, wuv_h, wob_h,
            out_h, out_ref, xbt, xb, ckv, wqb, wuk, wuv, wob, wq_s, wk_s, wv_s, sems, *, S, DM, H, DH, MEM, SEG, DC):
    NP = H // 2
    NSEG = S // SEG
    STRIDE = (NSEG - WARM) // NCHAIN
    NPASS = WARM + STRIDE
    scale = DH ** -0.5 * LOG2E
    xb, wq_s, wk_s, wv_s = _as_bf16(xb, wq_s, wk_s, wv_s)

    b_copies = [_Load(s, d, sems, 6 + i) for i, (s, d) in enumerate(
        [(c_h, ckv), (wuk_h, wuk), (wuv_h, wuv), (xb_h, xbt), (wqb_h, wqb), (wob_h, wob)])]

    def branch_a(xat, xa, xs, mem0, me, ms, wo, a_all, b_all, bt_all, a_sum):
        a_sum, = _as_bf16(a_sum)
        xa, xs, me, ms, a_all, b_all, bt_all = _as_bf16(xa, xs, me, ms, a_all, b_all, bt_all)

        def precompute(wq, wk, wv, hq, hk):
            hq, hk = _as_bf16(hq, hk)
            x_copy = _Load(xa_h, xat, sems, 0)
            qk_copies = [[_Load(s, d, sems, 12 + 2 * i + k, i * 64 * H, 64 * H)
                          for k, (s, d) in enumerate([(wq_h, wq), (wk_h, wk)])]
                         for i in range(DM // 64)]
            v_copies = [_Load(s, d, sems, 1 + i) for i, (s, d) in enumerate(
                [(wv_h, wv), (wo_h, wo), (mem0_h, mem0)])]
            x_copy.start()
            for cps in qk_copies:
                for cp in cps:
                    cp.start()
            x_copy.wait()

            def make_x(b, _):
                r0 = pl.multiple_of(b * TB, TB)
                xt = xat[:, pl.ds(r0, TB)]
                z = jnp.zeros((64, TB), BF)
                xa[pl.ds(r0, TB), :] = jnp.concatenate([xt, z], axis=0).T
                xs[pl.ds(r0, TB), :] = jnp.concatenate([z, xt], axis=0).T
            lax.fori_loop(0, S // TB, make_x, None)

            for i, cps in enumerate(qk_copies):
                for cp in cps:
                    cp.wait()
                if i == DM // 64 - 2:
                    for cp in v_copies:
                        cp.start()
                _split_heads(wq, hq, i * 64, 64)
                _split_heads(wk, hk, i * 64, 64)

            z = jnp.zeros((64, DH), BF)
            for j in range(NP):
                a0 = _dot_nt(hq[2 * j], jnp.concatenate([hk[2 * j], z], axis=0))
                a1 = _dot_nt(hq[2 * j + 1], jnp.concatenate([z, hk[2 * j + 1]], axis=0))
                a = _merge_pair(a0, a1) * scale
                a_all[j] = a.astype(BF)
                if j % 2:
                    zf = jnp.zeros((512 - DM, 2 * DM), F32)
                    b11, b12 = prev[0:256], a[0:256]
                    b21 = jnp.concatenate([prev[256:DM], zf], axis=0)
                    b22 = jnp.concatenate([a[256:DM], zf], axis=0)
                    for n, t in enumerate((b11 + b22, b12 - b22, b21 - b11, b11 + b12, b21 + b22)):
                        a_sum[j // 2, n] = t.astype(BF)
                prev = a
            for cp in v_copies:
                cp.wait()
            for cp in b_copies:
                cp.start()
            hv = hq
            for i in range(DM // 64):
                _split_heads(wv, hv, i * 64, 64)
            for j in range(NP):
                b0 = _dot_nt(hv[2 * j], jnp.concatenate([wo[2 * j], z], 0)).astype(BF)
                b1 = _dot_nt(hv[2 * j + 1], jnp.concatenate([wo[2 * j + 1], z], 0)).astype(BF)
                b = jnp.concatenate([b0, b1], axis=0)
                b_all[j] = b
                bt_all[j] = b.T[0:DM]

        raw = pltpu.VMEM((2 * DM * H, 128), BF)
        pl.run_scoped(precompute, raw, raw, raw,
                      _packed(H, DM, DH), _packed(H, DM, DH))

        def seg_keys(seg):
            r = pl.ds(pl.multiple_of(seg * SEG, SEG), SEG)
            return (jnp.concatenate([me[seg], xa[r, :]], axis=0),
                    jnp.concatenate([ms[seg], xs[r, :]], axis=0))

        tk = lax.broadcasted_iota(jnp.int32, (48, 128), 0)
        tcol = lax.broadcasted_iota(jnp.int32, (48, 128), 1)
        exists = (tk < MEM) | (tk >= 16)

        def softmax_t(s):
            p = jnp.exp2(s - jnp.max(s, axis=0, keepdims=True))
            return p * (1.0 / jnp.sum(p, axis=0, keepdims=True))

        def one_pass(t, carry):
            mem, spec = carry
            spec = jnp.where(t == WARM, mem, spec)
            sh = pltpu.roll(mem, 64, 1)
            z8 = jnp.zeros((8, 512), F32)
            for c in range(NCHAIN):
                seg = c * STRIDE + t
                me[seg] = jnp.concatenate([mem[8 * c:8 * c + 8], z8], 0).astype(BF)
                ms[seg] = jnp.concatenate([sh[8 * c:8 * c + 8], z8], 0).astype(BF)
            mb = mem[:, :DM].astype(BF)
            qs = [_dot(mb, a_all[j]) for j in range(NP)]
            kcs, ss = [], []
            for c in range(NCHAIN):
                ke, ko = seg_keys(c * STRIDE + t)
                z16 = jnp.zeros((16, 512), BF)
                kcs.append(jnp.concatenate([ke, z16, ko, z16], axis=0))
                lhs = jnp.concatenate(
                    [q[8 * c:8 * c + 8, 0:512] for q in qs]
                    + [q[8 * c:8 * c + 8, 384:896] for q in qs], axis=0).astype(BF)
                ss.append(_dot_nt(kcs[c], lhs))
            even = tcol < 64
            zp = jnp.zeros((16, 128), F32)
            ps = []
            for s in ss:
                p = softmax_t(jnp.where(exists, jnp.where(even, s[0:48], s[64:112]), NEG_PAD))
                ps.append(jnp.concatenate(
                    [jnp.where(even, p, 0.0), zp, jnp.where(even, 0.0, p), zp], 0).T.astype(BF))
            phs = []
            for c in range(NCHAIN):
                r = _dot(ps[c], kcs[c])
                phs.append([_merge_pair(r[8 * j:8 * j + 8], r[64 + 8 * j:72 + 8 * j])
                            for j in range(NP)])
            new = None
            for j in range(NP):
                l = jnp.concatenate([phs[c][j] for c in range(NCHAIN)], axis=0).astype(BF)
                d = _dot(l, b_all[j])
                new = d if new is None else new + d
            return new.astype(BF).astype(F32), spec

        def sweep(state):
            n, _, mem = state
            fin, spec = lax.fori_loop(jnp.where(n == 0, 0, WARM), NPASS, one_pass, (mem, mem))
            nxt = jnp.concatenate([spec[0:8], fin[0:8 * (NCHAIN - 1)]], axis=0)
            diff = pltpu.bitcast(nxt, jnp.int32) != pltpu.bitcast(spec, jnp.int32)
            return n + 1, jnp.max(diff.astype(jnp.int32)), nxt

        m0 = jnp.concatenate([mem0[...].astype(F32), jnp.zeros((MEM, 64), F32)], axis=1)
        lax.while_loop(lambda st: (st[0] < NCHAIN) & (st[1] > 0), sweep,
                       (jnp.int32(0), jnp.int32(1), jnp.concatenate([m0] * NCHAIN, axis=0)))

        visible = (tk < MEM) | ((tk >= 16) & (tk - 16 <= (tcol & (SEG - 1))))
        fill = jnp.where(exists, NEG_MASK, NEG_PAD).astype(F32)

        def probs_t(s):
            return softmax_t(jnp.where(visible, s, fill))

        for cp in b_copies:
            cp.wait()

        def tokens(qp, ph):
            qp, ph = _as_bf16(qp, ph)

            def tok_block(b, _):
                def project(u, g):
                    x = xa[pl.ds(pl.multiple_of((2 * b + u) * TB, TB), TB), :]
                    hb = TB // 2
                    a11, a12, a21, a22 = x[:hb, :256], x[:hb, 256:], x[hb:, :256], x[hb:, 256:]
                    m2 = _dot(_add(a21, a22), a_all[2 * g, 0:256, :])
                    m4 = _dot(a22, a_sum[g, 2])
                    qp[u, 2 * g, hb:TB, :] = (m2 + m4).astype(BF)
                    m5 = _dot(_add(a11, a12)[:, 0:DM - 256], a_all[2 * g + 1, 256:DM, :])
                    m3 = _dot(a11, a_sum[g, 1])
                    qp[u, 2 * g + 1, 0:hb, :] = (m3 + m5).astype(BF)
                    m1 = _dot(_add(a11, a22), a_sum[g, 0])
                    m7 = _dot(_add(a12, a22, -1), a_sum[g, 4])
                    qp[u, 2 * g, 0:hb, :] = ((m4 - m5) + m1 + m7).astype(BF)
                    m6 = _dot(_add(a21, a11, -1), a_sum[g, 3])
                    qp[u, 2 * g + 1, hb:TB, :] = ((m3 - m2) + m1 + m6).astype(BF)
                    return [d[0:8, c:c + 128] for d in (m2, m4, m5, m3, m1, m7, m6)
                            for c in (0, 384, 768)]

                def scores(u, g):
                    ke, ko = seg_keys((2 * b + u) * (TB // SEG) + g)
                    rows = slice(g * SEG, (g + 1) * SEG)
                    res = []
                    for j0 in range(0, NP, 4):
                        js = range(j0, j0 + 4)
                        res.append((
                            _dot_nt(ke, jnp.concatenate([qp[u, j, rows, 0:512] for j in js], 0)),
                            _dot_nt(ko, jnp.concatenate([qp[u, j, rows, 384:896] for j in js], 0))))
                    return res

                def probs(sc):
                    zp = jnp.zeros((16, 128), F32)
                    return [jnp.concatenate([probs_t(se), zp, probs_t(so), zp], 0).T.astype(BF)
                            for se, so in sc]

                def mix(u, g, ps):
                    ke, ko = seg_keys((2 * b + u) * (TB // SEG) + g)
                    z = jnp.zeros((48, 384), BF)
                    z16 = jnp.zeros((16, 2 * DM), BF)
                    kc = jnp.concatenate([jnp.concatenate([ke, z], axis=1), z16,
                                          jnp.concatenate([z, ko], axis=1), z16], axis=0)
                    r = _dot(jnp.concatenate(ps, axis=0), kc).astype(BF)
                    for j in range(NP):
                        ph[u, j, g * SEG:(g + 1) * SEG, :] = r[SEG * j:SEG * (j + 1)]

                def side(j, after):
                    m0 = pl.multiple_of(b * 128 + j * 16, 16)
                    _split_heads(wuk, wk_s, m0, 16, after)
                    _split_heads(wuv, wv_s, m0, 16, after)
                    mq = jnp.minimum(b, DM // 64 - 1) * 64 + j // 2 * 16
                    _split_heads(wqb, wq_s, pl.multiple_of(mq, 16), 16, after, (j % 2,))

                def emit(u, acc):
                    r = pl.ds(pl.multiple_of((2 * b + u) * TB, TB), TB)
                    z = jnp.zeros((64, TB), BF)
                    out_ref[r, 0:512] = jnp.concatenate([acc.astype(BF), z], axis=0).T
                    xb[r, :] = jnp.concatenate([xbt[:, r], z], axis=0).T

                for g in range(NP // 2):
                    pins = project(0, g)
                    side(2 * g, pins)
                    side(2 * g + 1, pins)
                for g in range(TB // SEG):
                    sc = scores(0, g)
                    project(1, g)
                    mix(0, g, probs(sc))
                acc = None
                for g in range(TB // SEG):
                    sc = scores(1, g)
                    for j in (2 * g, 2 * g + 1):
                        d = _dot_nt(bt_all[j], ph[0, j])
                        acc = d if acc is None else acc + d
                    mix(1, g, probs(sc))
                emit(0, acc)
                acc = None
                for j in range(NP):
                    d = _dot_nt(bt_all[j], ph[1, j])
                    acc = d if acc is None else acc + d
                emit(1, acc)
            lax.fori_loop(0, S // (2 * TB), tok_block, None)

        pl.run_scoped(tokens, _packed(2, NP, TB, 2 * DM), _packed(2, NP, TB, 2 * DM))

    pl.run_scoped(
        branch_a,
        pltpu.VMEM((DM, S), BF), _packed(S, 512), _packed(S, 512),
        pltpu.VMEM((MEM, DM), BF),
        _packed(NSEG, 16, 512), _packed(NSEG, 16, 512),
        pltpu.VMEM((H, DM, DH), BF),
        _packed(NP, DM, 2 * DM), _packed(NP, 2 * DM, 512),
        _packed(NP, DM, 2 * DM), _packed(NP // 2, 5, 256, 2 * DM))

    def branch_b(ctx, slot, k_s, v_s, cs):
        ctx, k_s, v_s, cs = _as_bf16(ctx, k_s, v_s, cs)
        qi = lax.broadcasted_iota(jnp.int32, (QB, QB // 2), 0)
        kj = lax.broadcasted_iota(jnp.int32, (QB, QB // 2), 1)
        causal = kj <= qi

        S2, C2, D2 = S // 2, DC // 2, DH // 2

        def latent_sums(i, _):
            r = pl.ds(pl.multiple_of(i * 128, 128), 128)
            r2 = pl.ds(pl.multiple_of(S2 + i * 128, 128), 128)
            a11, a12, a21, a22 = ckv[r, 0:C2], ckv[r, C2:DC], ckv[r2, 0:C2], ckv[r2, C2:DC]
            cs[0, r, :] = _add(a11, a22)
            cs[1, r, :] = _add(a21, a22)
            cs[2, r, :] = _add(a11, a12)
            cs[3, r, :] = _add(a21, a11, -1)
            cs[4, r, :] = _add(a12, a22, -1)
        lax.fori_loop(0, S2 // 128, latent_sums, None)

        def project_kv(h):
            def quad(i, j):
                r, c = slice(i * C2, (i + 1) * C2), slice(j * D2, (j + 1) * D2)
                return jnp.concatenate([wk_s[h, r, c], wv_s[h, r, c]], axis=1)

            def put(i, j, val):
                r, c = slice(i * S2, (i + 1) * S2), slice(j * D2, (j + 1) * D2)
                k_s[r, c] = val[:, 0:D2].astype(BF)
                v_s[r, c] = val[:, D2:DH].astype(BF)

            b11, b12, b21, b22 = quad(0, 0), quad(0, 1), quad(1, 0), quad(1, 1)
            m2 = _dot(cs[1], b11)
            m4 = _dot(ckv[S2:S, C2:DC], _add(b21, b11, -1))
            put(1, 0, m2 + m4)
            m5 = _dot(cs[2], b22)
            m3 = _dot(ckv[0:S2, 0:C2], _add(b12, b22, -1))
            put(0, 1, m3 + m5)
            m1 = _dot(cs[0], _add(b11, b22))
            put(0, 0, (m4 - m5) + m1 + _dot(cs[4], _add(b21, b22)))
            put(1, 1, (m3 - m2) + m1 + _dot(cs[3], _add(b11, b12)))

        def head(h, _):
            slot[h] = h
            hq = slot[h]
            ctx[hq] = (_dot(xb[:, 0:DM], wq_s[h]) * scale).astype(BF)
            project_kv(h)

            def scores(i):
                lo, mid, hi = i * QB, i * QB + QB // 2, (i + 1) * QB
                q = ctx[hq, lo:hi, :]
                return (_dot_nt(q, k_s[0:mid, :]), _dot_nt(q[QB // 2:], k_s[mid:hi, :]))

            def attend(i, sa, sb):
                lo, mid, hi = i * QB, i * QB + QB // 2, (i + 1) * QB
                cols = [sa[:, c:c + 128] for c in range(0, mid, 128)]
                cols[-1] = jnp.where(causal, cols[-1], NEG_MASK)
                sb = jnp.where(causal[0:QB // 2], sb, NEG_MASK)
                m = functools.reduce(jnp.maximum, cols)
                m = jnp.concatenate([m[:QB // 2], jnp.maximum(m[QB // 2:], sb)], axis=0)
                m = jnp.max(m, axis=-1, keepdims=True)
                cols = [jnp.exp2(c - m) for c in cols]
                pb = jnp.exp2(sb - m[QB // 2:])
                l = functools.reduce(jnp.add, cols)
                l = jnp.concatenate([l[:QB // 2], l[QB // 2:] + pb], axis=0)
                l = jnp.sum(l, axis=-1, keepdims=True)
                o = _dot(jnp.concatenate(cols, axis=1).astype(BF), v_s[0:mid, :])
                ob = _dot(pb.astype(BF), v_s[mid:hi, :])
                o = jnp.concatenate([o[:QB // 2], o[QB // 2:] + ob], axis=0)
                return (o * (1.0 / l)).astype(BF)

            nxt = scores(S // QB - 1)
            for i in reversed(range(S // QB)):
                cur = nxt
                if i:
                    nxt = scores(i - 1)
                if i < S // QB - 1:
                    ctx[h, (i + 1) * QB:(i + 2) * QB, :] = done
                done = attend(i, *cur)
            ctx[h, 0:QB, :] = done
        lax.fori_loop(0, H, head, None)

        lane = lax.broadcasted_iota(jnp.int32, (512, 128), 1)

        def store(i):
            r = pl.ds(pl.multiple_of(i * 512, 512), 512)
            return pltpu.make_async_copy(out_ref.at[r], out_h.at[r], sems.at[52 + i])

        def out_block(i, _):
            r = pl.ds(pl.multiple_of(i * 512, 512), 512)
            acc = None
            for h in range(H):
                d = _dot_nt(wob[h], ctx[h, r, :])
                acc = d if acc is None else acc + d
            res = jnp.concatenate([jnp.zeros((64, 512), BF), acc.astype(BF)], axis=0).T
            out_ref[r, 384:512] = jnp.where(lane < 64, out_ref[r, 384:512], res[:, 0:128])
            out_ref[r, 512:896] = res[:, 128:512]
            store(i).start()
        lax.fori_loop(0, S // 512, out_block, None)
        for i in range(S // 512):
            store(i).wait()

    pl.run_scoped(
        branch_b,
        _packed(H, S, DH), pltpu.SMEM((H,), jnp.int32),
        _packed(S, DH), _packed(S, DH), _packed(5, S // 2, DC // 2))


@functools.partial(jax.jit, static_argnames=("A_seg_len",))
def pallas_concat_heads__memory_aug_recurrent_mem_tr__compressed_kv_cla__prompt_kernel(
    A_x, A_mem0, A_Wq, A_Wk, A_Wv, A_Wo, A_seg_len,
    B_x, B_c_kv, B_w_q, B_w_uk, B_w_uv, B_w_o,
):
    _, S, DM = A_x.shape
    _, H, DH = A_Wq.shape
    MEM = A_mem0.shape[1]
    DC = B_c_kv.shape[2]
    assert (S, DM, H, DH, MEM, A_seg_len, DC) == (2048, 448, 16, 256, 8, 32, 1024)
    assert B_x.shape == A_x.shape and B_c_kv.shape[1] == S

    out = pl.pallas_call(
        functools.partial(_kernel, S=S, DM=DM, H=H, DH=DH, MEM=MEM, SEG=A_seg_len, DC=DC),
        out_shape=jax.ShapeDtypeStruct((S, 2 * DM), BF),
        in_specs=[pl.BlockSpec(memory_space=pl.ANY)] * 12,
        out_specs=pl.BlockSpec(memory_space=pl.ANY),
        scratch_shapes=[
            pltpu.VMEM((S, 2 * DM), BF),
            pltpu.VMEM((DM, S), BF), _packed(S, 512), pltpu.VMEM((S, DC), BF),
            pltpu.VMEM((2 * DM * H, 128), BF), pltpu.VMEM((2 * DC * H, 128), BF),
            pltpu.VMEM((2 * DC * H, 128), BF), pltpu.VMEM((H, DM, DH), BF),
            _packed(H, DM, DH), _packed(H, DC, DH), _packed(H, DC, DH),
            pltpu.SemaphoreType.DMA((56,)),
        ],
        compiler_params=pltpu.CompilerParams(vmem_limit_bytes=120 * 1024 * 1024),
    )(
        A_x.reshape(S, DM).T, A_mem0.reshape(MEM, DM),
        A_Wq.reshape(DM * H, DH), A_Wk.reshape(DM * H, DH), A_Wv.reshape(DM * H, DH),
        A_Wo.transpose(0, 2, 1),
        B_x.reshape(S, DM).T, B_c_kv.reshape(S, DC),
        B_w_q.reshape(DM * H, DH), B_w_uk.reshape(DC * H, DH), B_w_uv.reshape(DC * H, DH),
        B_w_o.transpose(0, 2, 1),
    )
    return out.reshape(1, S, 2 * DM)
```

```python
import functools
import math

import jax
import jax.numpy as jnp
from jax import lax
import jax.experimental.pallas as pl
import jax.experimental.pallas.tpu as pltpu

BF = jnp.bfloat16
F32 = jnp.float32
LOG2E = math.log2(math.e)
NEG_MASK = -1e9 * LOG2E
NEG_PAD = -3e38

NCHAIN = 4
WARM = 4
TB = 128
QB = 256


def _dot(a, b):
    return jnp.dot(a, b, preferred_element_type=F32)


def _dot_nt(a, b):
    return lax.dot_general(a, b, (((1,), (1,)), ((), ())), preferred_element_type=F32)


def _split_heads(raw_ref, dst_ref, m0, rows, after=None, halves=(0, 1)):
    half = raw_ref.shape[0] // 2
    g = rows // 8
    sub = lax.broadcasted_iota(jnp.int32, (g, 8, 128), 1)
    for i in halves:
        w = raw_ref[pl.ds(pl.multiple_of(i * half + m0 * 16, 128), rows * 16), :]
        w = pltpu.bitcast(w, jnp.uint32).reshape(g, 8, 8, 128)
        if after is not None:
            pins = jnp.stack([after.pop(0) for _ in range(g)])[:, None]
            w = w | ((pltpu.bitcast(pins, jnp.uint32) >> 31) >> 1)
        v = [w[:, m] for m in range(8)]
        for d in (4, 2, 1):
            keep = (sub & d) == 0
            for a in range(8):
                if not a & d:
                    x, y = v[a], v[a + d]
                    v[a] = jnp.where(keep, x, pltpu.roll(y, d, 1))
                    v[a + d] = jnp.where(keep, pltpu.roll(x, 8 - d, 1), y)
        for p in range(8):
            x = v[p].reshape(rows, 128)
            lo = pltpu.bitcast(x << 16, F32).astype(BF)
            hi = pltpu.bitcast(x & jnp.uint32(0xFFFF0000), F32).astype(BF)
            dst_ref[2 * p, pl.ds(m0, rows), 128 * i:128 * (i + 1)] = lo
            dst_ref[2 * p + 1, pl.ds(m0, rows), 128 * i:128 * (i + 1)] = hi


def _packed(*shape):
    return pltpu.VMEM(shape[:-2] + (shape[-2] // 2, shape[-1]), jnp.uint32)


def _as_bf16(*refs):
    return [r.bitcast(BF) for r in refs]


class _Load:
    def __init__(self, src, dst, sems, i, r0=0, rows=None):
        n = src.shape[0]
        rows = rows or n
        if dst.shape != src.shape:
            self.cps = [pltpu.make_async_copy(src.at[r0:r0 + rows, 128 * k:128 * (k + 1)],
                                              dst.at[k * n + r0:k * n + r0 + rows],
                                              sems.at[2 * i + k]) for k in range(2)]
        else:
            self.cps = [pltpu.make_async_copy(src, dst, sems.at[2 * i])]

    def start(self):
        for cp in self.cps:
            cp.start()

    def wait(self):
        for cp in self.cps:
            cp.wait()


def _add(x, y, sign=1):
    x, y = x.astype(F32), y.astype(F32)
    return (x + y if sign > 0 else x - y).astype(BF)


def _merge_pair(e, o):
    return jnp.concatenate([e[:, :384], e[:, 384:] + o[:, :128], o[:, 128:]], axis=1)


def _kernel(xa_h, mem0_h, wq_h, wk_h, wv_h, wo_h, xb_h, c_h, wqb_h, wuk_h, wuv_h, wob_h,
            out_h, out_ref, xbt, xb, ckv, wqb, wuk, wuv, wob, wq_s, wk_s, wv_s, sems,
            *, S, DM, H, DH, MEM, SEG, DC):
    NP = H // 2
    NSEG = S // SEG
    STRIDE = (NSEG - WARM) // NCHAIN
    NPASS = WARM + STRIDE
    scale = DH ** -0.5 * LOG2E
    xb, wq_s, wk_s, wv_s = _as_bf16(xb, wq_s, wk_s, wv_s)

    b_copies = [_Load(s, d, sems, 6 + i) for i, (s, d) in enumerate(
        [(c_h, ckv), (wuk_h, wuk), (wuv_h, wuv), (xb_h, xbt), (wqb_h, wqb), (wob_h, wob)])]

    def branch_a(xat, xa, xs, mem0, me, ms, wo, a_all, b_all, bt_all, a_sum):
        a_sum, = _as_bf16(a_sum)
        xa, xs, me, ms, a_all, b_all, bt_all = _as_bf16(xa, xs, me, ms, a_all, b_all, bt_all)

        def precompute(wq, wk, wv, hq, hk):
            hq, hk = _as_bf16(hq, hk)
            x_copy = _Load(xa_h, xat, sems, 0)
            qk_copies = [[_Load(s, d, sems, 12 + 2 * i + k, i * 64 * H, 64 * H)
                          for k, (s, d) in enumerate([(wq_h, wq), (wk_h, wk)])]
                         for i in range(DM // 64)]
            v_copies = [_Load(s, d, sems, 1 + i) for i, (s, d) in enumerate(
                [(wv_h, wv), (wo_h, wo), (mem0_h, mem0)])]
            x_copy.start()
            for cps in qk_copies:
                for cp in cps:
                    cp.start()
            x_copy.wait()

            def make_x(b, _):
                r0 = pl.multiple_of(b * TB, TB)
                xt = xat[:, pl.ds(r0, TB)]
                z = jnp.zeros((64, TB), BF)
                xa[pl.ds(r0, TB), :] = jnp.concatenate([xt, z], axis=0).T
                xs[pl.ds(r0, TB), :] = jnp.concatenate([z, xt], axis=0).T
            lax.fori_loop(0, S // TB, make_x, None)

            for i, cps in enumerate(qk_copies):
                for cp in cps:
                    cp.wait()
                if i == DM // 64 - 2:
                    for cp in v_copies:
                        cp.start()
                _split_heads(wq, hq, i * 64, 64)
                _split_heads(wk, hk, i * 64, 64)

            z = jnp.zeros((64, DH), BF)
            for j in range(NP):
                a0 = _dot_nt(hq[2 * j], jnp.concatenate([hk[2 * j], z], axis=0))
                a1 = _dot_nt(hq[2 * j + 1], jnp.concatenate([z, hk[2 * j + 1]], axis=0))
                a = _merge_pair(a0, a1) * scale
                a_all[j] = a.astype(BF)
                if j % 2:
                    zf = jnp.zeros((512 - DM, 2 * DM), F32)
                    b11, b12 = prev[0:256], a[0:256]
                    b21 = jnp.concatenate([prev[256:DM], zf], axis=0)
                    b22 = jnp.concatenate([a[256:DM], zf], axis=0)
                    for n, t in enumerate((b11 + b22, b12 - b22, b21 - b11, b11 + b12, b21 + b22)):
                        a_sum[j // 2, n] = t.astype(BF)
                prev = a
            for cp in v_copies:
                cp.wait()
            for cp in b_copies:
                cp.start()
            hv = hq
            for i in range(DM // 64):
                _split_heads(wv, hv, i * 64, 64)
            for j in range(NP):
                b0 = _dot_nt(hv[2 * j], jnp.concatenate([wo[2 * j], z], 0)).astype(BF)
                b1 = _dot_nt(hv[2 * j + 1], jnp.concatenate([wo[2 * j + 1], z], 0)).astype(BF)
                b = jnp.concatenate([b0, b1], axis=0)
                b_all[j] = b
                bt_all[j] = b.T[0:DM]

        raw = pltpu.VMEM((2 * DM * H, 128), BF)
        pl.run_scoped(precompute, raw, raw, raw,
                      _packed(H, DM, DH), _packed(H, DM, DH))

        def seg_keys(seg):
            r = pl.ds(pl.multiple_of(seg * SEG, SEG), SEG)
            return (jnp.concatenate([me[seg], xa[r, :]], axis=0),
                    jnp.concatenate([ms[seg], xs[r, :]], axis=0))

        tk = lax.broadcasted_iota(jnp.int32, (48, 128), 0)
        tcol = lax.broadcasted_iota(jnp.int32, (48, 128), 1)
        exists = (tk < MEM) | (tk >= 16)

        def softmax_t(s):
            p = jnp.exp2(s - jnp.max(s, axis=0, keepdims=True))
            return p * (1.0 / jnp.sum(p, axis=0, keepdims=True))

        def one_pass(t, carry):
            mem, spec = carry
            spec = jnp.where(t == WARM, mem, spec)
            sh = pltpu.roll(mem, 64, 1)
            z8 = jnp.zeros((8, 512), F32)
            for c in range(NCHAIN):
                seg = c * STRIDE + t
                me[seg] = jnp.concatenate([mem[8 * c:8 * c + 8], z8], 0).astype(BF)
                ms[seg] = jnp.concatenate([sh[8 * c:8 * c + 8], z8], 0).astype(BF)
            mb = mem[:, :DM].astype(BF)
            qs = [_dot(mb, a_all[j]) for j in range(NP)]
            kcs, ss = [], []
            for c in range(NCHAIN):
                ke, ko = seg_keys(c * STRIDE + t)
                z16 = jnp.zeros((16, 512), BF)
                kcs.append(jnp.concatenate([ke, z16, ko, z16], axis=0))
                lhs = jnp.concatenate(
                    [q[8 * c:8 * c + 8, 0:512] for q in qs]
                    + [q[8 * c:8 * c + 8, 384:896] for q in qs], axis=0).astype(BF)
                ss.append(_dot_nt(kcs[c], lhs))
            even = tcol < 64
            zp = jnp.zeros((16, 128), F32)
            ps = []
            for s in ss:
                p = softmax_t(jnp.where(exists, jnp.where(even, s[0:48], s[64:112]), NEG_PAD))
                ps.append(jnp.concatenate(
                    [jnp.where(even, p, 0.0), zp, jnp.where(even, 0.0, p), zp], 0).T.astype(BF))
            phs = []
            for c in range(NCHAIN):
                r = _dot(ps[c], kcs[c])
                phs.append([_merge_pair(r[8 * j:8 * j + 8], r[64 + 8 * j:72 + 8 * j])
                            for j in range(NP)])
            new = None
            for j in range(NP):
                l = jnp.concatenate([phs[c][j] for c in range(NCHAIN)], axis=0).astype(BF)
                d = _dot(l, b_all[j])
                new = d if new is None else new + d
            return new.astype(BF).astype(F32), spec

        def sweep(state):
            n, _, mem = state
            fin, spec = lax.fori_loop(jnp.where(n == 0, 0, WARM), NPASS, one_pass, (mem, mem))
            nxt = jnp.concatenate([spec[0:8], fin[0:8 * (NCHAIN - 1)]], axis=0)
            diff = pltpu.bitcast(nxt, jnp.int32) != pltpu.bitcast(spec, jnp.int32)
            return n + 1, jnp.max(diff.astype(jnp.int32)), nxt

        m0 = jnp.concatenate([mem0[...].astype(F32), jnp.zeros((MEM, 64), F32)], axis=1)
        lax.while_loop(lambda st: (st[0] < NCHAIN) & (st[1] > 0), sweep,
                       (jnp.int32(0), jnp.int32(1), jnp.concatenate([m0] * NCHAIN, axis=0)))

        visible = (tk < MEM) | ((tk >= 16) & (tk - 16 <= (tcol & (SEG - 1))))
        fill = jnp.where(exists, NEG_MASK, NEG_PAD).astype(F32)

        def probs_t(s):
            return softmax_t(jnp.where(visible, s, fill))

        for cp in b_copies:
            cp.wait()

        def tokens(qp, ph):
            qp, ph = _as_bf16(qp, ph)

            def tok_block(b, _):
                def project(u, g):
                    x = xa[pl.ds(pl.multiple_of((2 * b + u) * TB, TB), TB), :]
                    hb = TB // 2
                    a11, a12, a21, a22 = x[:hb, :256], x[:hb, 256:], x[hb:, :256], x[hb:, 256:]
                    m2 = _dot(_add(a21, a22), a_all[2 * g, 0:256, :])
                    m4 = _dot(a22, a_sum[g, 2])
                    qp[u, 2 * g, hb:TB, :] = (m2 + m4).astype(BF)
                    m5 = _dot(_add(a11, a12)[:, 0:DM - 256], a_all[2 * g + 1, 256:DM, :])
                    m3 = _dot(a11, a_sum[g, 1])
                    qp[u, 2 * g + 1, 0:hb, :] = (m3 + m5).astype(BF)
                    m1 = _dot(_add(a11, a22), a_sum[g, 0])
                    m7 = _dot(_add(a12, a22, -1), a_sum[g, 4])
                    qp[u, 2 * g, 0:hb, :] = ((m4 - m5) + m1 + m7).astype(BF)
                    m6 = _dot(_add(a21, a11, -1), a_sum[g, 3])
                    qp[u, 2 * g + 1, hb:TB, :] = ((m3 - m2) + m1 + m6).astype(BF)
                    return [d[0:8, c:c + 128] for d in (m2, m4, m5, m3, m1, m7, m6)
                            for c in (0, 384, 768)]

                def scores(u, g):
                    ke, ko = seg_keys((2 * b + u) * (TB // SEG) + g)
                    rows = slice(g * SEG, (g + 1) * SEG)
                    res = []
                    for j0 in range(0, NP, 4):
                        js = range(j0, j0 + 4)
                        res.append((
                            _dot_nt(ke, jnp.concatenate([qp[u, j, rows, 0:512] for j in js], 0)),
                            _dot_nt(ko, jnp.concatenate([qp[u, j, rows, 384:896] for j in js], 0))))
                    return res

                def probs(sc):
                    zp = jnp.zeros((16, 128), F32)
                    return [jnp.concatenate([probs_t(se), zp, probs_t(so), zp], 0).T.astype(BF)
                            for se, so in sc]

                def mix(u, g, ps):
                    ke, ko = seg_keys((2 * b + u) * (TB // SEG) + g)
                    z = jnp.zeros((48, 384), BF)
                    z16 = jnp.zeros((16, 2 * DM), BF)
                    kc = jnp.concatenate([jnp.concatenate([ke, z], axis=1), z16,
                                          jnp.concatenate([z, ko], axis=1), z16], axis=0)
                    r = _dot(jnp.concatenate(ps, axis=0), kc).astype(BF)
                    for j in range(NP):
                        ph[u, j, g * SEG:(g + 1) * SEG, :] = r[SEG * j:SEG * (j + 1)]

                def side(j, after):
                    m0 = pl.multiple_of(b * 128 + j * 16, 16)
                    _split_heads(wuk, wk_s, m0, 16, after)
                    _split_heads(wuv, wv_s, m0, 16, after)
                    mq = jnp.minimum(b, DM // 64 - 1) * 64 + j // 2 * 16
                    _split_heads(wqb, wq_s, pl.multiple_of(mq, 16), 16, after, (j % 2,))

                def emit(u, acc):
                    r = pl.ds(pl.multiple_of((2 * b + u) * TB, TB), TB)
                    z = jnp.zeros((64, TB), BF)
                    out_ref[r, 0:512] = jnp.concatenate([acc.astype(BF), z], axis=0).T
                    xb[r, :] = jnp.concatenate([xbt[:, r], z], axis=0).T

                for g in range(NP // 2):
                    pins = project(0, g)
                    side(2 * g, pins)
                    side(2 * g + 1, pins)
                for g in range(TB // SEG):
                    sc = scores(0, g)
                    project(1, g)
                    mix(0, g, probs(sc))
                acc = None
                for g in range(TB // SEG):
                    sc = scores(1, g)
                    for j in (2 * g, 2 * g + 1):
                        d = _dot_nt(bt_all[j], ph[0, j])
                        acc = d if acc is None else acc + d
                    mix(1, g, probs(sc))
                emit(0, acc)
                acc = None
                for j in range(NP):
                    d = _dot_nt(bt_all[j], ph[1, j])
                    acc = d if acc is None else acc + d
                emit(1, acc)
            lax.fori_loop(0, S // (2 * TB), tok_block, None)

        pl.run_scoped(tokens, _packed(2, NP, TB, 2 * DM), _packed(2, NP, TB, 2 * DM))

    pl.run_scoped(
        branch_a,
        pltpu.VMEM((DM, S), BF), _packed(S, 512), _packed(S, 512),
        pltpu.VMEM((MEM, DM), BF),
        _packed(NSEG, 16, 512), _packed(NSEG, 16, 512),
        pltpu.VMEM((H, DM, DH), BF),
        _packed(NP, DM, 2 * DM), _packed(NP, 2 * DM, 512),
        _packed(NP, DM, 2 * DM), _packed(NP // 2, 5, 256, 2 * DM))

    def branch_b(ctx, slot, k_s, v_s, cs, xsum, ws):
        ctx, k_s, v_s, cs, xsum, ws = _as_bf16(ctx, k_s, v_s, cs, xsum, ws)
        qi = lax.broadcasted_iota(jnp.int32, (QB, QB // 2), 0)
        kj = lax.broadcasted_iota(jnp.int32, (QB, QB // 2), 1)
        causal = kj <= qi

        S2, C2, D2 = S // 2, DC // 2, DH // 2

        def latent_sums(i, _):
            r = pl.ds(pl.multiple_of(i * 128, 128), 128)
            r2 = pl.ds(pl.multiple_of(S2 + i * 128, 128), 128)
            a11, a12, a21, a22 = ckv[r, 0:C2], ckv[r, C2:DC], ckv[r2, 0:C2], ckv[r2, C2:DC]
            cs[0, r, :] = _add(a11, a22)
            cs[1, r, :] = _add(a21, a22)
            cs[2, r, :] = _add(a11, a12)
            cs[3, r, :] = _add(a21, a11, -1)
            cs[4, r, :] = _add(a12, a22, -1)
            a11, a12, a21, a22 = xb[r, 0:256], xb[r, 256:512], xb[r2, 0:256], xb[r2, 256:512]
            xsum[0, r, :] = _add(a11, a22)
            xsum[1, r, :] = _add(a21, a22)
            xsum[2, r, :] = _add(a11, a12)
            xsum[3, r, :] = _add(a21, a11, -1)
            xsum[4, r, :] = _add(a12, a22, -1)
        lax.fori_loop(0, S2 // 128, latent_sums, None)

        def project_kv(h):
            def quad(i, j):
                r, c = slice(i * C2, (i + 1) * C2), slice(j * D2, (j + 1) * D2)
                return jnp.concatenate([wk_s[h, r, c], wv_s[h, r, c]], axis=1)

            def put(i, j, val):
                r, c = slice(i * S2, (i + 1) * S2), slice(j * D2, (j + 1) * D2)
                k_s[r, c] = val[:, 0:D2].astype(BF)
                v_s[r, c] = val[:, D2:DH].astype(BF)

            b11, b12, b21, b22 = quad(0, 0), quad(0, 1), quad(1, 0), quad(1, 1)
            m2 = _dot(cs[1], b11)
            m4 = _dot(ckv[S2:S, C2:DC], _add(b21, b11, -1))
            put(1, 0, m2 + m4)
            m5 = _dot(cs[2], b22)
            m3 = _dot(ckv[0:S2, 0:C2], _add(b12, b22, -1))
            put(0, 1, m3 + m5)
            m1 = _dot(cs[0], _add(b11, b22))
            put(0, 0, (m4 - m5) + m1 + _dot(cs[4], _add(b21, b22)))
            put(1, 1, (m3 - m2) + m1 + _dot(cs[3], _add(b11, b12)))

        def project_q(h, hq):
            z = jnp.zeros((512 - DM, D2), BF)
            b11, b12 = wq_s[h, 0:256, 0:D2], wq_s[h, 0:256, D2:DH]
            b21 = jnp.concatenate([wq_s[h, 256:DM, 0:D2], z], axis=0)
            b22 = jnp.concatenate([wq_s[h, 256:DM, D2:DH], z], axis=0)

            def put(i, j, val):
                ctx[hq, i * S2:(i + 1) * S2, j * D2:(j + 1) * D2] = (val * scale).astype(BF)

            m2 = _dot(xsum[1], b11)
            m4 = _dot(xb[S2:S, 256:512], _add(b21, b11, -1))
            put(1, 0, m2 + m4)
            m5 = _dot(xsum[2], b22)
            m3 = _dot(xb[0:S2, 0:256], _add(b12, b22, -1))
            put(0, 1, m3 + m5)
            m1 = _dot(xsum[0], _add(b11, b22))
            put(0, 0, (m4 - m5) + m1 + _dot(xsum[4], _add(b21, b22)))
            put(1, 1, (m3 - m2) + m1 + _dot(xsum[3], _add(b11, b12)))

        def head(h, _):
            slot[h] = h
            hq = slot[h]
            project_q(h, hq)
            project_kv(h)

            def scores(i):
                lo, mid, hi = i * QB, i * QB + QB // 2, (i + 1) * QB
                q = ctx[hq, lo:hi, :]
                return (_dot_nt(q, k_s[0:mid, :]), _dot_nt(q[QB // 2:], k_s[mid:hi, :]))

            def attend(i, sa, sb):
                lo, mid, hi = i * QB, i * QB + QB // 2, (i + 1) * QB
                cols = [sa[:, c:c + 128] for c in range(0, mid, 128)]
                cols[-1] = jnp.where(causal, cols[-1], NEG_MASK)
                sb = jnp.where(causal[0:QB // 2], sb, NEG_MASK)
                m = functools.reduce(jnp.maximum, cols)
                m = jnp.concatenate([m[:QB // 2], jnp.maximum(m[QB // 2:], sb)], axis=0)
                m = jnp.max(m, axis=-1, keepdims=True)
                cols = [jnp.exp2(c - m) for c in cols]
                pb = jnp.exp2(sb - m[QB // 2:])
                l = functools.reduce(jnp.add, cols)
                l = jnp.concatenate([l[:QB // 2], l[QB // 2:] + pb], axis=0)
                l = jnp.sum(l, axis=-1, keepdims=True)
                o = _dot(jnp.concatenate(cols, axis=1).astype(BF), v_s[0:mid, :])
                ob = _dot(pb.astype(BF), v_s[mid:hi, :])
                o = jnp.concatenate([o[:QB // 2], o[QB // 2:] + ob], axis=0)
                return (o * (1.0 / l)).astype(BF)

            nxt = scores(S // QB - 1)
            for i in reversed(range(S // QB)):
                cur = nxt
                if i:
                    nxt = scores(i - 1)
                if i < S // QB - 1:
                    ctx[h, (i + 1) * QB:(i + 2) * QB, :] = done
                done = attend(i, *cur)
            ctx[h, 0:QB, :] = done
        lax.fori_loop(0, H, head, None)

        lane = lax.broadcasted_iota(jnp.int32, (512, 128), 1)

        def store(i):
            r = pl.ds(pl.multiple_of(i * 512, 512), 512)
            return pltpu.make_async_copy(out_ref.at[r], out_h.at[r], sems.at[52 + i])

        M2 = DM // 2

        def wo_sums(h, _):
            a11, a12 = wob[h, 0:M2, :], wob[h + H // 2, 0:M2, :]
            a21, a22 = wob[h, M2:DM, :], wob[h + H // 2, M2:DM, :]
            ws[h, 0] = _add(a11, a22)
            ws[h, 1] = _add(a21, a22)
            ws[h, 2] = _add(a11, a12)
            ws[h, 3] = _add(a21, a11, -1)
            ws[h, 4] = _add(a12, a22, -1)
        lax.fori_loop(0, H // 2, wo_sums, None)

        def out_block(i, _):
            r = pl.ds(pl.multiple_of(i * 512, 512), 512)
            r1 = pl.ds(pl.multiple_of(i * 512, 512), 256)
            r2 = pl.ds(pl.multiple_of(i * 512 + 256, 256), 256)
            m = [None] * 7
            for h in range(H // 2):
                b11, b12 = ctx[h, r1, :], ctx[h, r2, :]
                b21, b22 = ctx[h + H // 2, r1, :], ctx[h + H // 2, r2, :]
                ops = ((ws[h, 0], _add(b11, b22)), (ws[h, 1], b11),
                       (wob[h, 0:M2, :], _add(b12, b22, -1)),
                       (wob[h + H // 2, M2:DM, :], _add(b21, b11, -1)), (ws[h, 2], b22),
                       (ws[h, 3], _add(b11, b12)), (ws[h, 4], _add(b21, b22)))
                for n, (x, y) in enumerate(ops):
                    d = _dot_nt(x, y)
                    m[n] = d if m[n] is None else m[n] + d
            m1, m2, m3, m4, m5, m6, m7 = m
            acc = jnp.concatenate([jnp.concatenate([m1 + m4 - m5 + m7, m3 + m5], axis=1),
                                   jnp.concatenate([m2 + m4, m1 - m2 + m3 + m6], axis=1)], axis=0)
            res = jnp.concatenate([jnp.zeros((64, 512), BF), acc.astype(BF)], axis=0).T
            out_ref[r, 384:512] = jnp.where(lane < 64, out_ref[r, 384:512], res[:, 0:128])
            out_ref[r, 512:896] = res[:, 128:512]
            store(i).start()
        lax.fori_loop(0, S // 512, out_block, None)
        for i in range(S // 512):
            store(i).wait()

    pl.run_scoped(
        branch_b,
        _packed(H, S, DH), pltpu.SMEM((H,), jnp.int32),
        _packed(S, DH), _packed(S, DH), _packed(5, S // 2, DC // 2),
        _packed(5, S // 2, 256), _packed(H // 2, 5, DM // 2, DH))


@functools.partial(jax.jit, static_argnames=("A_seg_len",))
def pallas_concat_heads__memory_aug_recurrent_mem_tr__compressed_kv_cla__prompt_kernel(
    A_x, A_mem0, A_Wq, A_Wk, A_Wv, A_Wo, A_seg_len,
    B_x, B_c_kv, B_w_q, B_w_uk, B_w_uv, B_w_o,
):
    _, S, DM = A_x.shape
    _, H, DH = A_Wq.shape
    MEM = A_mem0.shape[1]
    DC = B_c_kv.shape[2]
    assert (S, DM, H, DH, MEM, A_seg_len, DC) == (2048, 448, 16, 256, 8, 32, 1024)
    assert B_x.shape == A_x.shape and B_c_kv.shape[1] == S

    out = pl.pallas_call(
        functools.partial(_kernel, S=S, DM=DM, H=H, DH=DH, MEM=MEM, SEG=A_seg_len, DC=DC),
        out_shape=jax.ShapeDtypeStruct((S, 2 * DM), BF),
        in_specs=[pl.BlockSpec(memory_space=pl.ANY)] * 12,
        out_specs=pl.BlockSpec(memory_space=pl.ANY),
        scratch_shapes=[
            pltpu.VMEM((S, 2 * DM), BF),
            pltpu.VMEM((DM, S), BF), _packed(S, 512), pltpu.VMEM((S, DC), BF),
            pltpu.VMEM((2 * DM * H, 128), BF), pltpu.VMEM((2 * DC * H, 128), BF),
            pltpu.VMEM((2 * DC * H, 128), BF), pltpu.VMEM((H, DM, DH), BF),
            _packed(H, DM, DH), _packed(H, DC, DH), _packed(H, DC, DH),
            pltpu.SemaphoreType.DMA((56,)),
        ],
        compiler_params=pltpu.CompilerParams(vmem_limit_bytes=120 * 1024 * 1024),
    )(
        A_x.reshape(S, DM).T, A_mem0.reshape(MEM, DM),
        A_Wq.reshape(DM * H, DH), A_Wk.reshape(DM * H, DH), A_Wv.reshape(DM * H, DH),
        A_Wo.transpose(0, 2, 1),
        B_x.reshape(S, DM).T, B_c_kv.reshape(S, DC),
        B_w_q.reshape(DM * H, DH), B_w_uk.reshape(DC * H, DH), B_w_uv.reshape(DC * H, DH),
        B_w_o.transpose(0, 2, 1),
    )
    return out.reshape(1, S, 2 * DM)
```
